```python
import jax
import jax.numpy as jnp

def _softmax(x, axis=-1):
    return jax.nn.softmax(x, axis=axis)

def _gelu(x):
    return jax.nn.gelu(x, approximate=True)

def _silu(x):
    return jax.nn.silu(x)

def _sigmoid(x):
    return jax.nn.sigmoid(x)

def _layernorm(x, axis=-1, eps=1e-05):
    m = jnp.mean(x, axis=axis, keepdims=True)
    v = jnp.var(x, axis=axis, keepdims=True)
    return (x - m) / jnp.sqrt(v + eps)

def _scatter_add(tgt, idx, src, axis=0):
    return tgt.at[idx].add(src)

def _segment_sum(src, seg, n):
    return jax.ops.segment_sum(src, seg, n)

class _Rng:

    def __init__(self, key):
        self._k = key

    def _next(self):
        self._k, sub = jax.random.split(self._k)
        return sub

    def normal(self, shape):
        return jax.random.normal(self._next(), shape, dtype=jnp.bfloat16)

    def randint(self, lo, hi, shape):
        return jax.random.randint(self._next(), shape, lo, hi, dtype=jnp.int32)

    def uniform(self, shape, lo=0.0, hi=1.0):
        return jax.random.uniform(self._next(), shape, jnp.bfloat16, lo, hi)

    def permutation(self, n):
        return jax.random.permutation(self._next(), n)
kernel_name = 'interleave_layers__memory_aug_recurrent_mem_tr__linear_kernel_hedgehog__prompt'

def setup_inputs():
    _rng = _Rng(jax.random.key(int.from_bytes(__import__("os").urandom(4), "little")))
    _w = lambda a: (lambda t: t.astype(jnp.bfloat16) if jnp.issubdtype(t.dtype, jnp.floating) else t)(jnp.asarray(a))

    def _A_setup():
        B, S, Dm = (1, 2048, 640)
        H, Dh = (32, 192)
        M, seg = (8, 32)
        seg = min(seg, S)
        S = S // seg * seg
        return {'x': _w((lambda *s: _rng.normal(s) * 0.05)(B, S, Dm)), 'mem0': _w((lambda *s: _rng.normal(s) * 0.05)(B, M, Dm)), 'Wq': _w((lambda *s: _rng.normal(s) * 0.05)(Dm, H, Dh) * Dm ** (-0.5)), 'Wk': _w((lambda *s: _rng.normal(s) * 0.05)(Dm, H, Dh) * Dm ** (-0.5)), 'Wv': _w((lambda *s: _rng.normal(s) * 0.05)(Dm, H, Dh) * Dm ** (-0.5)), 'Wo': _w((lambda *s: _rng.normal(s) * 0.05)(H, Dh, Dm) * (H * Dh) ** (-0.5)), 'seg_len': seg}
    _A_in = _A_setup()

    def _B_setup():
        B, S, D, H = (1, 2048, 640, 32)
        Dh = D // H
        return {'x': _w((lambda *s: _rng.normal(s) * 0.05)(B, S, D)), 'wqkv': _w((lambda *s: _rng.normal(s) * 0.05)(D, 3 * D)), 'w_phi': _w((lambda *s: _rng.normal(s) * 0.05)(H, Dh, Dh) * Dh ** (-0.5)), 'wo': _w((lambda *s: _rng.normal(s) * 0.05)(D, D))}
    _B_in = _B_setup()
    return {'A_x': _A_in['x'], 'A_mem0': _A_in['mem0'], 'A_Wq': _A_in['Wq'], 'A_Wk': _A_in['Wk'], 'A_Wv': _A_in['Wv'], 'A_Wo': _A_in['Wo'], 'A_seg_len': _A_in['seg_len'], 'B_x': _B_in['x'], 'B_wqkv': _B_in['wqkv'], 'B_w_phi': _B_in['w_phi'], 'B_wo': _B_in['wo']}

def reference(A_x, A_mem0, A_Wq, A_Wk, A_Wv, A_Wo, A_seg_len, B_x, B_wqkv, B_w_phi, B_wo):

    def _A_ref(x, mem0, Wq, Wk, Wv, Wo, seg_len):
        B, S, Dm = x.shape
        H, Dh = (Wq.shape[1], Wq.shape[2])
        M = mem0.shape[1]
        scale = Dh ** (-0.5)
        n_seg = S // seg_len
        L = M + seg_len
        idx = jnp.arange(L)
        mask = (idx[:, None] < M) | (idx[:, None] >= idx[None, :])
        mem = mem0
        outs = []
        for s in range(n_seg):
            xs = x[:, s * seg_len:(s + 1) * seg_len, :].copy()
            h = jnp.concatenate([mem, xs], axis=1)
            q = jnp.einsum('btd,dhe->bhte', h, Wq)
            k = jnp.einsum('btd,dhe->bhte', h, Wk)
            v = jnp.einsum('btd,dhe->bhte', h, Wv)
            scores = jnp.einsum('bhqe,bhke->bhqk', q, k) * scale
            scores = jnp.where(mask[None, None], scores, -1000000000.0)
            p = _softmax(scores, axis=-1)
            o = jnp.einsum('bhqk,bhke->bhqe', p, v)
            o = jnp.einsum('bhte,hed->btd', o, Wo)
            mem = o[:, :M, :].copy()
            outs.append(o[:, M:, :])
        return jnp.concatenate(outs, axis=1)

    def _B_ref(x, wqkv, w_phi, wo):
        B, S, D = x.shape
        H = 32
        Dh = D // H
        qkv = (lambda x, *d: x.transpose(*d))((x @ wqkv).reshape(B, S, 3, H, Dh), 2, 0, 3, 1, 4)
        q, k, v = (qkv[0], qkv[1], qkv[2])
        pq = jnp.einsum('bhsd,hdf->bhsf', q, w_phi)
        pk = jnp.einsum('bhsd,hdf->bhsf', k, w_phi)
        phi_q = jnp.concatenate([_softmax(pq, axis=-1), _softmax(-pq, axis=-1)], axis=-1)
        phi_k = jnp.concatenate([_softmax(pk, axis=-1), _softmax(-pk, axis=-1)], axis=-1)
        kv = jnp.einsum('bhsf,bhsd->bhfd', phi_k, v)
        z = jnp.einsum('bhsf->bhf', phi_k)
        num = jnp.einsum('bhqf,bhfd->bhqd', phi_q, kv)
        den = jnp.einsum('bhqf,bhf->bhq', phi_q, z)[..., None] + 1e-06
        o = num / den
        return (lambda x, *d: x.transpose(*d))(o, 0, 2, 1, 3).reshape(B, S, D) @ wo
    x = A_x
    x = x + _A_ref(_layernorm(x, axis=-1), A_mem0, A_Wq, A_Wk, A_Wv, A_Wo, A_seg_len)
    x = x + _B_ref(_layernorm(x, axis=-1), B_wqkv, B_w_phi, B_wo)
    x = x + _A_ref(_layernorm(x, axis=-1), A_mem0, A_Wq, A_Wk, A_Wv, A_Wo, A_seg_len)
    x = x + _B_ref(_layernorm(x, axis=-1), B_wqkv, B_w_phi, B_wo)
    return x
```

```python
import jax
import jax.numpy as jnp
from jax import lax
import jax.experimental.pallas as pl
import jax.experimental.pallas.tpu as pltpu

_BF = jnp.bfloat16
_F32 = jnp.float32
_NN = (((1,), (0,)), ((), ()))
_NT = (((1,), (1,)), ((), ()))
_LANES = 128
_SUB = 8
_EPS = 1e-05

_RING = 4
_CHUNK = 256


def _mm(a, b, dims=_NN):
    return lax.dot_general(a, b, dims, preferred_element_type=_F32)


def _iota(shape, dim):
    return lax.broadcasted_iota(jnp.int32, shape, dim)


def _layernorm(x):
    m = jnp.mean(x, axis=-1, keepdims=True)
    c = x - m
    v = jnp.mean(c * c, axis=-1, keepdims=True)
    return c * lax.rsqrt(v + _EPS)


def _make_kernel(S, D, M, SEG, H, DH, HB):
    L = M + SEG
    NSEG = S // SEG
    NP = H // 2
    PW = 2 * DH
    FB = D // HB
    NG = HB // _SUB
    GR = FB * _SUB
    NCH = S // _CHUNK
    scale = DH ** (-0.5)
    split_tile = DH // _LANES
    split_lane = DH % _LANES

    def expand(t):
        zero = jnp.zeros((L, _LANES), _F32)
        in_a = _iota((L, _LANES), 1) < split_lane
        top, bot = [], []
        for j in range(PW // _LANES):
            blk = t[:, j * _LANES:(j + 1) * _LANES]
            if j < split_tile:
                top.append(blk)
                bot.append(zero)
            elif j == split_tile:
                top.append(jnp.where(in_a, blk, 0.0))
                bot.append(jnp.where(in_a, 0.0, blk))
            else:
                top.append(zero)
                bot.append(blk)
        both = [jnp.concatenate(top, axis=1), jnp.concatenate(bot, axis=1)]
        return jnp.concatenate(both, axis=0).astype(_BF)

    def pair_softmax(s):
        row = _iota((L, 2 * L), 0)
        col = _iota((L, 2 * L), 1)
        is_a = col < L
        key = jnp.where(is_a, col, col - L)
        s = jnp.where((row < M) | (row >= key), s * scale, -1000000000.0)
        max_a = jnp.max(jnp.where(is_a, s, -jnp.inf), axis=1, keepdims=True)
        max_b = jnp.max(jnp.where(is_a, -jnp.inf, s), axis=1, keepdims=True)
        e = jnp.exp(s - jnp.where(is_a, max_a, max_b))
        sum_a = jnp.sum(jnp.where(is_a, e, 0.0), axis=1, keepdims=True)
        sum_b = jnp.sum(jnp.where(is_a, 0.0, e), axis=1, keepdims=True)
        return e / jnp.where(is_a, sum_a, sum_b)

    def feature_map(p):
        rows = [p[f * _SUB:(f + 1) * _SUB] for f in range(FB)]
        hi, lo = rows[0], rows[0]
        for r in rows[1:]:
            hi = jnp.maximum(hi, r)
            lo = jnp.minimum(lo, r)
        out = []
        for es in ([jnp.exp(r - hi) for r in rows], [jnp.exp(lo - r) for r in rows]):
            tot = es[0]
            for e in es[1:]:
                tot = tot + e
            inv = 1.0 / tot
            out += [e * inv for e in es]
        return jnp.concatenate(out, axis=0)

    def kernel(x_hbm, mem0_ref, wq_hbm, wk_hbm, wv_hbm, wo_hbm, bqkv_hbm, phi_ref, bwo_hbm,
               out_hbm,
               wqk, wv, wo, stage, xio, xs, xb, xn, p_scr, o_scr,
               bqkv_in, bwo_in, bw, bwo, phiq, kv_acc, kvm,
               stage_sem, misc_sem, out_sem):

        x_cp = pltpu.make_async_copy(x_hbm, xio, misc_sem.at[0])
        wo_cp = pltpu.make_async_copy(wo_hbm, wo, misc_sem.at[1])
        bqkv_cp = pltpu.make_async_copy(bqkv_hbm, bqkv_in, misc_sem.at[2])
        bwo_cp = pltpu.make_async_copy(bwo_hbm, bwo_in, misc_sem.at[3])

        def stage_cps(g, slot):
            rows = pl.ds(pl.multiple_of(g * PW, PW), PW)
            return [pltpu.make_async_copy(src.at[rows], stage.at[slot, i], stage_sem.at[slot, i])
                    for i, src in enumerate((wq_hbm, wk_hbm, wv_hbm))]

        for g in range(_RING - 1):
            for cp in stage_cps(g, g):
                cp.start()

        def load_pair(g, carry):
            nxt = g + _RING - 1

            @pl.when(nxt < NP)
            def _():
                for cp in stage_cps(nxt, nxt % _RING):
                    cp.start()

            @pl.when(nxt == NP)
            def _():
                x_cp.start()
                wo_cp.start()

            slot = g % _RING
            for cp in stage_cps(g, slot):
                cp.wait()
            wqk[g, :, :PW] = stage[slot, 0].T
            wqk[g, :, PW:] = stage[slot, 1].T
            wv[g] = stage[slot, 2].T
            return carry

        lax.fori_loop(0, NP, load_pair, 0)
        x_cp.wait()

        def init_x(c, carry):
            rows = pl.ds(pl.multiple_of(c * _CHUNK, _CHUNK), _CHUNK)
            xs[rows, :] = xio[rows, :].astype(_F32)
            return carry

        lax.fori_loop(0, NCH, init_x, 0)
        wo_cp.wait()
        bqkv_cp.start()
        bwo_cp.start()

        def prep_b_weights():
            bqkv_cp.wait()
            bwo_cp.wait()
            head = _iota((HB, D), 0)
            col = _iota((HB, D), 1)
            t = None
            for d in range(FB):
                sel = (col == head * FB + d).astype(_BF)
                part = _mm(phi_ref[d], sel)
                t = part if t is None else t + part
            sub = _iota((_SUB, D), 0)
            col = _iota((_SUB, D), 1)
            for g in range(NG):
                first = (g * _SUB + sub) * FB
                own = (col >= first) & (col < first + FB)
                phi_t = jnp.concatenate(
                    [jnp.where(own, t[f:f + 1, :], 0.0) for f in range(FB)], axis=0)
                perm = jnp.concatenate(
                    [(col == first + d).astype(_F32) for d in range(FB)], axis=0)
                lo = g * GR // _LANES * _LANES
                hi = -(-(g + 1) * GR // _LANES) * _LANES
                for part, lhs in enumerate((phi_t, phi_t, perm)):
                    w = bqkv_in[:, part * D + lo:part * D + hi]
                    bw[part, g * GR:(g + 1) * GR, :] = _mm(lhs[:, lo:hi], w, _NT).astype(_BF)
                bwo[g * GR:(g + 1) * GR, :] = _mm(perm[:, lo:hi], bwo_in[lo:hi, :]).astype(_BF)

        def seg_rows(s):
            return pl.ds(pl.multiple_of(s * SEG, SEG), SEG)

        def a_step(s, mem):
            h = jnp.concatenate([mem, xn[s % 2]], axis=0)
            xn[(s + 1) % 2] = _layernorm(xs[seg_rows(jnp.minimum(s + 1, NSEG - 1)), :])
            prev = seg_rows(jnp.maximum(s - 1, 0))
            xb[prev, :] = _layernorm(xs[prev, :]).astype(_BF)

            cur = _mm(h, wqk[0])
            for g in range(NP):
                nxt = _mm(h, wqk[g + 1]) if g + 1 < NP else _mm(h, wv[0])
                p_scr[g] = pair_softmax(_mm(cur[:, :PW], expand(cur[:, PW:]), _NT))
                cur = nxt
            for g in range(NP):
                if g + 1 < NP:
                    nxt = _mm(h, wv[g + 1])
                o_scr[:, g * PW:(g + 1) * PW] = _mm(p_scr[g], expand(cur))
                cur = nxt
            out = _mm(o_scr[...], wo[...])
            xs[seg_rows(s), :] = xs[seg_rows(s), :] + out[M:]
            return out[:M]

        def layer_a():
            xn[0] = _layernorm(xs[0:SEG, :])
            lax.fori_loop(0, NSEG, a_step, mem0_ref[...].astype(_F32))
            xb[S - SEG:S, :] = _layernorm(xs[S - SEG:S, :]).astype(_BF)

        def chunk_rows(c):
            return pl.ds(pl.multiple_of(c * _CHUNK, _CHUNK), _CHUNK)

        def b_pass1(c, carry):
            xc = xb[chunk_rows(c), :]
            ones = jnp.ones((_SUB, _CHUNK), _F32)
            for g in range(NG):
                grp = slice(g * GR, (g + 1) * GR)
                pk = _mm(bw[1, grp, :], xc, _NT)
                v = _mm(bw[2, grp, :], xc, _NT)
                pq = _mm(bw[0, grp, :], xc, _NT)
                phik = feature_map(pk).astype(_BF)
                kv_acc[g] = kv_acc[g] + _mm(jnp.concatenate([v, ones], axis=0), phik, _NT)
                phiq[c, g] = feature_map(pq).astype(_BF)
            return carry

        def out_cp(c):
            return pltpu.make_async_copy(xio.at[chunk_rows(c)], out_hbm.at[chunk_rows(c)],
                                         out_sem.at[c])

        def layer_b(last):
            kv_acc[...] = jnp.zeros(kv_acc.shape, _F32)
            lax.fori_loop(0, NCH, b_pass1, 0)
            shape = (GR + _SUB, 2 * GR)
            same_head = (_iota(shape, 0) % _SUB) == (_iota(shape, 1) % _SUB)
            for g in range(NG):
                kvm[g] = jnp.where(same_head, kv_acc[g], 0.0)

            def b_pass2(c, carry):
                outs = []
                for g in range(NG):
                    nd = _mm(kvm[g], phiq[c, g])
                    inv = 1.0 / (nd[GR:] + 1e-06)
                    outs += [nd[d * _SUB:(d + 1) * _SUB] * inv for d in range(FB)]
                o = jnp.concatenate(outs, axis=0).T
                y = xs[chunk_rows(c), :] + _mm(o, bwo[...])
                xs[chunk_rows(c), :] = y
                xio[chunk_rows(c), :] = y.astype(_BF)

                @pl.when(last)
                def _():
                    out_cp(c).start()

                return carry

            lax.fori_loop(0, NCH, b_pass2, 0)

        def layer_pair(i, carry):
            layer_a()
            pl.when(i == 0)(prep_b_weights)
            layer_b(i == 1)
            return carry

        lax.fori_loop(0, 2, layer_pair, 0)
        for c in range(NCH):
            out_cp(c).wait()

    scratch = [
        pltpu.VMEM((NP, D, 2 * PW), _BF),
        pltpu.VMEM((NP, D, PW), _BF),
        pltpu.VMEM((NP * PW, D), _BF),
        pltpu.VMEM((_RING, 3, PW, D), _BF),
        pltpu.VMEM((S, D), _BF),
        pltpu.VMEM((S, D), _F32),
        pltpu.VMEM((S, D), _BF),
        pltpu.VMEM((2, SEG, D), _F32),
        pltpu.VMEM((NP, L, 2 * L), _F32),
        pltpu.VMEM((L, NP * PW), _F32),
        pltpu.VMEM((D, 3 * D), _BF),
        pltpu.VMEM((D, D), _BF),
        pltpu.VMEM((3, D, D), _BF),
        pltpu.VMEM((D, D), _BF),
        pltpu.VMEM((NCH, NG, 2 * GR, _CHUNK), _BF),
        pltpu.VMEM((NG, GR + _SUB, 2 * GR), _F32),
        pltpu.VMEM((NG, GR + _SUB, 2 * GR), _F32),
        pltpu.SemaphoreType.DMA((_RING, 3)),
        pltpu.SemaphoreType.DMA((4,)),
        pltpu.SemaphoreType.DMA((NCH,)),
    ]
    return kernel, scratch


def pallas_interleave_layers__memory_aug_recurrent_mem_tr__linear_kernel_hedgehog__prompt_kernel(
    A_x, A_mem0, A_Wq, A_Wk, A_Wv, A_Wo, A_seg_len, B_x, B_wqkv, B_w_phi, B_wo,
):
    del B_x
    _, S, D = A_x.shape
    M = A_mem0.shape[1]
    _, H, DH = A_Wq.shape
    HB = B_w_phi.shape[0]
    kernel, scratch = _make_kernel(S, D, M, int(A_seg_len), H, DH, HB)

    def head_major(w):
        return jnp.transpose(w, (1, 2, 0)).reshape(H * DH, D)

    hbm = pl.BlockSpec(memory_space=pl.ANY)
    vmem = pl.BlockSpec(memory_space=pltpu.VMEM)
    out = pl.pallas_call(
        kernel,
        out_shape=jax.ShapeDtypeStruct((S, D), A_x.dtype),
        in_specs=[hbm, vmem, hbm, hbm, hbm, hbm, hbm, vmem, hbm],
        out_specs=hbm,
        scratch_shapes=scratch,
        compiler_params=pltpu.CompilerParams(vmem_limit_bytes=112 * 1024 * 1024),
    )(
        A_x.reshape(S, D),
        A_mem0.reshape(M, D),
        head_major(A_Wq),
        head_major(A_Wk),
        head_major(A_Wv),
        A_Wo.reshape(H * DH, D),
        B_wqkv,
        jnp.transpose(B_w_phi, (1, 2, 0)),
        B_wo,
    )
    return out.reshape(A_x.shape)
```

```python
import jax
import jax.numpy as jnp
from jax import lax
import jax.experimental.pallas as pl
import jax.experimental.pallas.tpu as pltpu

_BF = jnp.bfloat16
_F32 = jnp.float32
_U32 = jnp.uint32
_NN = (((1,), (0,)), ((), ()))
_NT = (((1,), (1,)), ((), ()))
_LANES = 128
_SUB = 8
_EPS = 1e-05
_LOG2E = 1.4426950408889634

_RING = 4
_CHUNK = 256
_LIGHT = 40
_UNROLL = 2
_UNROLL_LIGHT = 2
_LAG = 2
_UNROLL_B = 1


def _mm(a, b, dims=_NN):
    return lax.dot_general(a, b, dims, preferred_element_type=_F32)


def _iota(shape, dim):
    return lax.broadcasted_iota(jnp.int32, shape, dim)


def _pack(x):
    return pltpu.bitcast(x.astype(_BF), _U32)


def _unpack(x):
    return pltpu.bitcast(x, _BF)


def _layernorm(x):
    m = jnp.mean(x, axis=-1, keepdims=True)
    c = x - m
    v = jnp.mean(c * c, axis=-1, keepdims=True)
    return c * lax.rsqrt(v + _EPS)


def _make_kernel(S, D, M, SEG, H, DH, HB):
    L = M + SEG
    NSEG = S // SEG
    NP = H // 2
    PW = 2 * DH
    FB = D // HB
    NG = HB // 2
    GR = 2 * FB
    BLK = 4 * GR
    NCH = S // _CHUNK
    SPC = _CHUNK // SEG
    KEEP = SEG - _SUB
    scale = DH ** (-0.5)
    split_tile = DH // _LANES
    split_lane = DH % _LANES

    def expand(t):
        zero = jnp.zeros((L, _LANES), _F32)
        in_a = _iota((L, _LANES), 1) < split_lane
        top, bot = [], []
        for j in range(PW // _LANES):
            blk = t[:, j * _LANES:(j + 1) * _LANES]
            if j < split_tile:
                top.append(blk)
                bot.append(zero)
            elif j == split_tile:
                top.append(jnp.where(in_a, blk, 0.0))
                bot.append(jnp.where(in_a, 0.0, blk))
            else:
                top.append(zero)
                bot.append(blk)
        both = [jnp.concatenate(top, axis=1), jnp.concatenate(bot, axis=1)]
        return jnp.concatenate(both, axis=0).astype(_BF)

    def pair_softmax(s):
        row = _iota((L, 2 * L), 0)
        col = _iota((L, 2 * L), 1)
        is_a = col < L
        key = jnp.where(is_a, col, col - L)
        s = jnp.where((row < M) | (row >= key), s * scale, -1000000000.0)
        max_a = jnp.max(jnp.where(is_a, s, -jnp.inf), axis=1, keepdims=True)
        max_b = jnp.max(jnp.where(is_a, -jnp.inf, s), axis=1, keepdims=True)
        e = jnp.exp(s - jnp.where(is_a, max_a, max_b))
        sum_a = jnp.sum(jnp.where(is_a, e, 0.0), axis=1, keepdims=True)
        sum_b = jnp.sum(jnp.where(is_a, 0.0, e), axis=1, keepdims=True)
        return e / jnp.where(is_a, sum_a, sum_b)

    def over_features(op, rows):
        r = rows[0]
        for t in rows[1:]:
            r = op(r, t)
        r = op(r, pltpu.roll(r, 4, 0))
        return op(r, pltpu.roll(r, 2, 0))

    def feature_map(p):
        rows = [p[i * _SUB:(i + 1) * _SUB] for i in range(GR // _SUB)]
        hi = over_features(jnp.maximum, rows)
        lo = over_features(jnp.minimum, rows)
        out = []
        for es in ([jnp.exp2(r - hi) for r in rows], [jnp.exp2(lo - r) for r in rows]):
            inv = 1.0 / over_features(jnp.add, es)
            out += [e * inv for e in es]
        return jnp.concatenate(out, axis=0)

    def kernel(x_hbm, mem0_ref, wq_hbm, wk_hbm, wv_hbm, wo_hbm, bqkv_hbm, phi_ref, bwo_hbm,
               out_hbm,
               wqk, wv, wo, stage, xtail, xpre, pre, xio, xs, xb, xn, mem_scr, p_scr, o_scr,
               bqkv_in, bwo_in, bw, bwo, phiq, kv_acc, ob,
               stage_sem, misc_sem, out_sem):

        tail_cp = pltpu.make_async_copy(
            x_hbm.at[pl.ds(0, _LIGHT), pl.ds(KEEP, _SUB)], xtail, misc_sem.at[0])
        x_cp = pltpu.make_async_copy(x_hbm, xio, misc_sem.at[1])
        bqkv_cp = pltpu.make_async_copy(bqkv_hbm, bqkv_in, misc_sem.at[2])
        bwo_cp = pltpu.make_async_copy(bwo_hbm, bwo_in, misc_sem.at[3])

        def stage_cps(g, slot):
            rows = pl.ds(pl.multiple_of(g * PW, PW), PW)
            return [pltpu.make_async_copy(src.at[rows], stage.at[slot, i], stage_sem.at[slot, i])
                    for i, src in enumerate((wq_hbm, wk_hbm, wv_hbm, wo_hbm))]

        tail_cp.start()
        for g in range(_RING - 1):
            for cp in stage_cps(g, g):
                cp.start()
        tail_cp.wait()
        xpre[...] = _pack(_layernorm(xtail[...].astype(_F32).reshape(_LIGHT * _SUB, D)))

        def load_pair(g, carry):
            nxt = g + _RING - 1

            @pl.when(nxt < NP)
            def _():
                for cp in stage_cps(nxt, nxt % _RING):
                    cp.start()

            @pl.when(nxt == NP)
            def _():
                x_cp.start()

            slot = g % _RING
            for cp in stage_cps(g, slot):
                cp.wait()
            lhs = _unpack(xpre[...])
            for i in range(3):
                pre[g, :, i * PW:(i + 1) * PW] = _mm(lhs, stage[slot, i], _NT)
            wqk[g, :, :PW] = _pack(stage[slot, 0].T)
            wqk[g, :, PW:] = _pack(stage[slot, 1].T)
            wv[g] = _pack(stage[slot, 2].T)
            wo[g] = _pack(stage[slot, 3])
            return carry

        with jax.named_scope("load"):
            lax.fori_loop(0, NP, load_pair, 0)
        x_cp.wait()
        bqkv_cp.start()
        bwo_cp.start()

        def init_x(c, carry):
            segs = pl.ds(c * SPC, SPC)
            xs[segs] = xio[segs].astype(_F32)
            return carry

        with jax.named_scope("initx"):
            lax.fori_loop(0, NCH, init_x, 0)

        def prep_b_weights():
            bqkv_cp.wait()
            bwo_cp.wait()
            head = _iota((HB, D), 0)
            col = _iota((HB, D), 1)
            t = None
            for d in range(FB):
                sel = jnp.where(col == head * FB + d, 1.0, 0.0).astype(_BF)
                part = _mm(phi_ref[d].astype(_F32), sel)
                t = part if t is None else t + part
            dup = jnp.where(_iota((GR, FB), 0) // 2 == _iota((GR, FB), 1), 1.0, 0.0)
            t = _mm(dup, t.astype(_BF))
            row = _iota((GR, D), 0)
            off = _iota((GR, D), 1) - (row % 2) * FB
            for b in range(D // BLK):
                lo = b * BLK // _LANES * _LANES
                hi = -(-(b + 1) * BLK // _LANES) * _LANES
                phi_t, perm = [], []
                for g in range(b * BLK // GR, (b + 1) * BLK // GR):
                    d = off - g * GR
                    phi_t.append(jnp.where((d >= 0) & (d < FB), t, 0.0)[:, lo:hi])
                    perm.append(jnp.where(d == row // 2, 1.0, 0.0)[:, lo:hi])
                phi_t = jnp.concatenate(phi_t, axis=0)
                perm = jnp.concatenate(perm, axis=0)
                rows = slice(b * BLK // 2, (b + 1) * BLK // 2)
                for part, (lhs, mul) in enumerate(((phi_t, _LOG2E), (phi_t, _LOG2E), (perm, 1.0))):
                    w = bqkv_in[:, part * D + lo:part * D + hi]
                    bw[part, rows, :] = _pack(_mm(lhs, w, _NT) * mul)
                bwo[rows, :] = _pack(_mm(perm, bwo_in[lo:hi, :]))

        def xb_rows(s, n):
            return pl.ds(pl.multiple_of(s * (SEG // 2), SEG // 2), n * (SEG // 2))

        def a_step(s, mem, light):
            if light:
                h = jnp.concatenate([mem, xn[s % 2, :KEEP]], axis=0).astype(_BF)
                tail = pl.ds(pl.multiple_of(s * _SUB, _SUB), _SUB)
                full = lambda r, g, a, b: jnp.concatenate([r, pre[g, tail, a:b]], axis=0)
            else:
                h = jnp.concatenate([mem, xn[s % 2]], axis=0)
                full = lambda r, g, a, b: r
            xn[(s + 1) % 2] = _layernorm(xs[jnp.minimum(s + 1, NSEG - 1)])
            prev = jnp.maximum(s - 1, 0)
            xb[xb_rows(prev, 1), :] = _pack(_layernorm(xs[prev]))

            cur = None
            for k in range(D // _LANES):
                w = _unpack(wqk[0, k * _LANES // 2:(k + 1) * _LANES // 2, :])
                part = _mm(h[:, k * _LANES:(k + 1) * _LANES], w)
                cur = part if cur is None else cur + part
            for g in range(NP):
                nxt = _mm(h, _unpack(wqk[g + 1] if g + 1 < NP else wv[0]))
                cur = full(cur, g, 0, 2 * PW)
                p_scr[g] = pair_softmax(_mm(cur[:, :PW], expand(cur[:, PW:]), _NT))
                cur = nxt
            out = None
            for g in range(NP + _LAG):
                if g + 1 < NP:
                    nxt = _mm(h, _unpack(wv[g + 1]))
                if g < NP:
                    o_scr[g] = _mm(p_scr[g], expand(full(cur, g, 2 * PW, 3 * PW)))
                    cur = nxt
                if g >= _LAG:
                    part = _mm(o_scr[g - _LAG], _unpack(wo[g - _LAG]))
                    out = part if out is None else out + part
            xs[s] = xs[s] + out[M:]
            return out[:M]

        def a_steps(lo, hi, light, unroll):
            def body(i, carry):
                mem = mem_scr[...]
                for u in range(unroll):
                    mem = a_step(i * unroll + u, mem, light)
                mem_scr[...] = mem
                return carry

            lax.fori_loop(lo // unroll, hi // unroll, body, 0)

        def layer_a(n_light):
            xn[0] = _layernorm(xs[0])
            mem_scr[...] = mem0_ref[...].astype(_F32)
            with jax.named_scope("alight"):
                a_steps(0, n_light, True, _UNROLL_LIGHT)
            with jax.named_scope("aloop"):
                a_steps(n_light, NSEG, False, _UNROLL)
            xb[(S - SEG) // 2:, :] = _pack(_layernorm(xs[NSEG - 1]))

        def b_pass1(c, carry):
            xc = _unpack(xb[xb_rows(c * SPC, SPC), :])
            ones = jnp.ones((_SUB, _CHUNK), _F32)

            def project(part, b):
                return _mm(_unpack(bw[part, b * BLK // 2:(b + 1) * BLK // 2, :]), xc, _NT)

            def groups(t):
                return [t[i * GR:(i + 1) * GR] for i in range(BLK // GR)]

            phik, vs = [], []
            for b in range(D // BLK):
                phik += [feature_map(p).astype(_BF) for p in groups(project(1, b))]
            for b in range(D // BLK):
                vs += groups(project(2, b))
            for b in range(D // BLK):
                for i, p in enumerate(groups(project(0, b))):
                    phiq[c, b * (BLK // GR) + i] = _pack(feature_map(p))
            for g in range(NG):
                kv_acc[g] = kv_acc[g] + _mm(jnp.concatenate([vs[g], ones], axis=0), phik[g], _NT)
            return carry

        def out_cp(c):
            segs = pl.ds(c * SPC, SPC)
            return pltpu.make_async_copy(xio.at[segs], out_hbm.at[segs], out_sem.at[c])

        def b_pass2(c, carry):
            outs = []
            for g in range(NG):
                nd = _mm(kv_acc[g], _unpack(phiq[c, g]))
                inv = 1.0 / (nd[GR:] + 1e-06)
                outs += [nd[i * _SUB:(i + 1) * _SUB] * inv for i in range(GR // _SUB)]
            ob[xb_rows(c * SPC, SPC), :] = _pack(jnp.concatenate(outs, axis=0).T)
            return carry

        def layer_b(last):
            kv_acc[...] = jnp.zeros(kv_acc.shape, _F32)
            with jax.named_scope("b1"):
                lax.fori_loop(0, NCH, b_pass1, 0, unroll=_UNROLL_B)
            shape = (GR + _SUB, 2 * GR)
            same_head = (_iota(shape, 0) % 2) == (_iota(shape, 1) % 2)
            for g in range(NG):
                kv_acc[g] = jnp.where(same_head, kv_acc[g], 0.0)
            with jax.named_scope("b2"):
                lax.fori_loop(0, NCH, b_pass2, 0, unroll=_UNROLL_B)

            def b_pass3(c, carry):
                segs = pl.ds(c * SPC, SPC)
                y = _mm(_unpack(ob[xb_rows(c * SPC, SPC), :]), _unpack(bwo[...]))
                y = xs[segs] + y.reshape(SPC, SEG, D)
                xs[segs] = y
                xio[segs] = y.astype(_BF)

                @pl.when(last)
                def _():
                    out_cp(c).start()

                return carry

            with jax.named_scope("b3"):
                lax.fori_loop(0, NCH, b_pass3, 0)

        def layer_pair(i, carry):
            layer_a(jnp.where(i == 0, _LIGHT, 0))
            with jax.named_scope("prep"):
                pl.when(i == 0)(prep_b_weights)
            layer_b(i == 1)
            return carry

        lax.fori_loop(0, 2, layer_pair, 0)
        for c in range(NCH):
            out_cp(c).wait()

    scratch = [
        pltpu.VMEM((NP, D // 2, 2 * PW), _U32),
        pltpu.VMEM((NP, D // 2, PW), _U32),
        pltpu.VMEM((NP, PW // 2, D), _U32),
        pltpu.VMEM((_RING, 4, PW, D), _BF),
        pltpu.VMEM((_LIGHT, _SUB, D), _BF),
        pltpu.VMEM((_LIGHT * _SUB // 2, D), _U32),
        pltpu.VMEM((NP, _LIGHT * _SUB, 3 * PW), _F32),
        pltpu.VMEM((NSEG, SEG, D), _BF),
        pltpu.VMEM((NSEG, SEG, D), _F32),
        pltpu.VMEM((S // 2, D), _U32),
        pltpu.VMEM((2, SEG, D), _F32),
        pltpu.VMEM((M, D), _F32),
        pltpu.VMEM((NP, L, 2 * L), _F32),
        pltpu.VMEM((NP, L, PW), _F32),
        pltpu.VMEM((D, 3 * D), _BF),
        pltpu.VMEM((D, D), _BF),
        pltpu.VMEM((3, D // 2, D), _U32),
        pltpu.VMEM((D // 2, D), _U32),
        pltpu.VMEM((NCH, NG, GR, _CHUNK), _U32),
        pltpu.VMEM((NG, GR + _SUB, 2 * GR), _F32),
        pltpu.VMEM((S // 2, D), _U32),
        pltpu.SemaphoreType.DMA((_RING, 4)),
        pltpu.SemaphoreType.DMA((4,)),
        pltpu.SemaphoreType.DMA((NCH,)),
    ]
    return kernel, scratch


def pallas_interleave_layers__memory_aug_recurrent_mem_tr__linear_kernel_hedgehog__prompt_kernel(
    A_x, A_mem0, A_Wq, A_Wk, A_Wv, A_Wo, A_seg_len, B_x, B_wqkv, B_w_phi, B_wo,
):
    del B_x
    _, S, D = A_x.shape
    M = A_mem0.shape[1]
    _, H, DH = A_Wq.shape
    HB = B_w_phi.shape[0]
    SEG = int(A_seg_len)
    kernel, scratch = _make_kernel(S, D, M, SEG, H, DH, HB)

    def head_major(w):
        return jnp.transpose(w, (1, 2, 0)).reshape(H * DH, D)

    hbm = pl.BlockSpec(memory_space=pl.ANY)
    vmem = pl.BlockSpec(memory_space=pltpu.VMEM)
    out = pl.pallas_call(
        kernel,
        out_shape=jax.ShapeDtypeStruct((S // SEG, SEG, D), A_x.dtype),
        in_specs=[hbm, vmem, hbm, hbm, hbm, hbm, hbm, vmem, hbm],
        out_specs=hbm,
        scratch_shapes=scratch,
        compiler_params=pltpu.CompilerParams(vmem_limit_bytes=120 * 1024 * 1024),
    )(
        A_x.reshape(S // SEG, SEG, D),
        A_mem0.reshape(M, D),
        head_major(A_Wq),
        head_major(A_Wk),
        head_major(A_Wv),
        A_Wo.reshape(H * DH, D),
        B_wqkv,
        jnp.transpose(B_w_phi, (1, 2, 0)),
        B_wo,
    )
    return out.reshape(A_x.shape)
```

```python
import jax
import jax.numpy as jnp
from jax import lax
import jax.experimental.pallas as pl
import jax.experimental.pallas.tpu as pltpu

_BF = jnp.bfloat16
_F32 = jnp.float32
_U32 = jnp.uint32
_NN = (((1,), (0,)), ((), ()))
_NT = (((1,), (1,)), ((), ()))
_LANES = 128
_SUB = 8
_EPS = 1e-05
_LOG2E = 1.4426950408889634

_RING = 4
_CHUNK = 256
_LIGHT = 40
_UNROLL = 2
_UNROLL_LIGHT = 2
_LAG = 2
_UNROLL_B = 2


def _mm(a, b, dims=_NN):
    return lax.dot_general(a, b, dims, preferred_element_type=_F32)


def _iota(shape, dim):
    return lax.broadcasted_iota(jnp.int32, shape, dim)


def _pack(x):
    return pltpu.bitcast(x.astype(_BF), _U32)


def _unpack(x):
    return pltpu.bitcast(x, _BF)


def _layernorm(x):
    m = jnp.mean(x, axis=-1, keepdims=True)
    c = x - m
    v = jnp.mean(c * c, axis=-1, keepdims=True)
    return c * lax.rsqrt(v + _EPS)


def _make_kernel(S, D, M, SEG, H, DH, HB):
    L = M + SEG
    NSEG = S // SEG
    NP = H // 2
    PW = 2 * DH
    FB = D // HB
    NG = HB // 2
    GR = 2 * FB
    BLK = 4 * GR
    NCH = S // _CHUNK
    SPC = _CHUNK // SEG
    SPI = 2 * _UNROLL_LIGHT
    KEEP = SEG - _SUB
    scale = DH ** (-0.5)
    split_tile = DH // _LANES
    split_lane = DH % _LANES

    def expand(t):
        zero = jnp.zeros((L, _LANES), _F32)
        in_a = _iota((L, _LANES), 1) < split_lane
        top, bot = [], []
        for j in range(PW // _LANES):
            blk = t[:, j * _LANES:(j + 1) * _LANES]
            if j < split_tile:
                top.append(blk)
                bot.append(zero)
            elif j == split_tile:
                top.append(jnp.where(in_a, blk, 0.0))
                bot.append(jnp.where(in_a, 0.0, blk))
            else:
                top.append(zero)
                bot.append(blk)
        both = [jnp.concatenate(top, axis=1), jnp.concatenate(bot, axis=1)]
        return jnp.concatenate(both, axis=0).astype(_BF)

    def pair_softmax(s):
        row = _iota((L, 2 * L), 0)
        col = _iota((L, 2 * L), 1)
        is_a = col < L
        key = jnp.where(is_a, col, col - L)
        s = jnp.where((row < M) | (row >= key), s * scale, -1000000000.0)
        max_a = jnp.max(jnp.where(is_a, s, -jnp.inf), axis=1, keepdims=True)
        max_b = jnp.max(jnp.where(is_a, -jnp.inf, s), axis=1, keepdims=True)
        e = jnp.exp(s - jnp.where(is_a, max_a, max_b))
        sum_a = jnp.sum(jnp.where(is_a, e, 0.0), axis=1, keepdims=True)
        sum_b = jnp.sum(jnp.where(is_a, 0.0, e), axis=1, keepdims=True)
        return e / jnp.where(is_a, sum_a, sum_b)

    def over_features(op, rows):
        r = rows[0]
        for t in rows[1:]:
            r = op(r, t)
        r = op(r, pltpu.roll(r, 4, 0))
        return op(r, pltpu.roll(r, 2, 0))

    def feature_map(p):
        rows = [p[i * _SUB:(i + 1) * _SUB] for i in range(GR // _SUB)]
        hi = over_features(jnp.maximum, rows)
        lo = over_features(jnp.minimum, rows)
        out = []
        for es in ([jnp.exp2(r - hi) for r in rows], [jnp.exp2(lo - r) for r in rows]):
            inv = 1.0 / over_features(jnp.add, es)
            out += [e * inv for e in es]
        return jnp.concatenate(out, axis=0)

    def kernel(x_hbm, mem0_ref, wq_hbm, wk_hbm, wv_hbm, wo_hbm, bqkv_hbm, phi_ref, bwo_hbm,
               out_hbm,
               wqk, wv, wo, stage, xtail, xpre, pre, xio, xs, xb, xn, mem_scr, p_scr, o_scr,
               bqkv_in, bwo_in, bw, bwo, phiq, kv_acc, ob,
               stage_sem, misc_sem, out_sem):

        tail_cp = pltpu.make_async_copy(
            x_hbm.at[pl.ds(0, _LIGHT), pl.ds(KEEP, _SUB)], xtail, misc_sem.at[0])
        head, rest = pl.ds(0, 2 * SPI), pl.ds(2 * SPI, NSEG - 2 * SPI)
        head_cp = pltpu.make_async_copy(x_hbm.at[head], xio.at[head], misc_sem.at[3])
        rest_cp = pltpu.make_async_copy(x_hbm.at[rest], xio.at[rest], misc_sem.at[4])
        bqkv_cp = pltpu.make_async_copy(bqkv_hbm, bqkv_in, misc_sem.at[1])
        bwo_cp = pltpu.make_async_copy(bwo_hbm, bwo_in, misc_sem.at[2])

        def stage_cps(g, slot):
            rows = pl.ds(pl.multiple_of(g * PW, PW), PW)
            return [pltpu.make_async_copy(src.at[rows], stage.at[slot, i], stage_sem.at[slot, i])
                    for i, src in enumerate((wq_hbm, wk_hbm, wv_hbm, wo_hbm))]

        tail_cp.start()
        for cp in stage_cps(0, 0):
            cp.start()
        with jax.named_scope("tailwait"):
            tail_cp.wait()
        xpre[...] = _pack(_layernorm(xtail[...].astype(_F32).reshape(_LIGHT * _SUB, D)))
        for g in range(1, _RING - 1):
            for cp in stage_cps(g, g):
                cp.start()

        def load_pair(g, carry):
            nxt = g + _RING - 1

            @pl.when(nxt < NP)
            def _():
                for cp in stage_cps(nxt, nxt % _RING):
                    cp.start()

            @pl.when(nxt == NP)
            def _():
                head_cp.start()

            slot = g % _RING
            for cp in stage_cps(g, slot):
                cp.wait()
            wo[g] = _pack(stage[slot, 3])
            lhs = _unpack(xpre[...])
            pre[g, :, :_LANES] = _mm(lhs, stage[slot, 0, :_LANES], _NT)
            w = stage[slot, 0].T
            wqk[g, :, :PW] = _pack(w)
            pre[g, :, _LANES:PW] = _mm(lhs, w[:, _LANES:])
            w = stage[slot, 1].T
            wqk[g, :, PW:] = _pack(w)
            pre[g, :, PW:2 * PW] = _mm(lhs, w)
            w = stage[slot, 2].T
            wv[g] = _pack(w)
            pre[g, :, 2 * PW:] = _mm(lhs, w)
            return carry

        with jax.named_scope("load"):
            lax.fori_loop(0, NP, load_pair, 0)
        rest_cp.start()
        bqkv_cp.start()
        bwo_cp.start()
        head_cp.wait()
        xs[0:SPI] = xio[0:SPI].astype(_F32)

        def prep_b_weights():
            bqkv_cp.wait()
            bwo_cp.wait()
            head = _iota((HB, D), 0)
            col = _iota((HB, D), 1)
            t = None
            for d in range(FB):
                sel = jnp.where(col == head * FB + d, 1.0, 0.0).astype(_BF)
                part = _mm(phi_ref[d].astype(_F32), sel)
                t = part if t is None else t + part
            dup = jnp.where(_iota((GR, FB), 0) // 2 == _iota((GR, FB), 1), 1.0, 0.0)
            t = _mm(dup, t.astype(_BF))
            off = _iota((GR, D), 1) - (_iota((GR, D), 0) % 2) * FB
            phi_t = [jnp.where((off >= g * GR) & (off < g * GR + FB), t, 0.0) for g in range(NG)]
            bw[2] = _pack(bqkv_in[:, 2 * D:].T)
            bwo[...] = _pack(bwo_in[...])
            for part in range(2):
                acc = [None] * NG
                for j in range(D // _LANES):
                    lo, hi = j * _LANES, (j + 1) * _LANES
                    gs = range(lo // GR, (hi - 1) // GR + 1)
                    lhs = jnp.concatenate([phi_t[g][:, lo:hi] for g in gs], axis=0)
                    r = _mm(lhs, bqkv_in[:, part * D + lo:part * D + hi], _NT)
                    for i, g in enumerate(gs):
                        piece = r[i * GR:(i + 1) * GR]
                        acc[g] = piece if acc[g] is None else acc[g] + piece
                bw[part] = _pack(jnp.concatenate(acc, axis=0) * _LOG2E)

        def xb_rows(s, n):
            return pl.ds(pl.multiple_of(s * (SEG // 2), SEG // 2), n * (SEG // 2))

        def a_step(s, mem, light):
            if light:
                h = jnp.concatenate([mem, xn[s % 2, :KEEP]], axis=0).astype(_BF)
                tail = pl.ds(pl.multiple_of(s * _SUB, _SUB), _SUB)
                full = lambda r, g, a, b: jnp.concatenate([r, pre[g, tail, a:b]], axis=0)
            else:
                h = jnp.concatenate([mem, xn[s % 2]], axis=0)
                full = lambda r, g, a, b: r
            xn[(s + 1) % 2] = _layernorm(xs[jnp.minimum(s + 1, NSEG - 1)])
            prev = jnp.maximum(s - 1, 0)
            xb[xb_rows(prev, 1), :] = _pack(_layernorm(xs[prev]))

            cur = None
            for k in range(D // _LANES):
                w = _unpack(wqk[0, k * _LANES // 2:(k + 1) * _LANES // 2, :])
                part = _mm(h[:, k * _LANES:(k + 1) * _LANES], w)
                cur = part if cur is None else cur + part
            for g in range(NP):
                nxt = _mm(h, _unpack(wqk[g + 1] if g + 1 < NP else wv[0]))
                cur = full(cur, g, 0, 2 * PW)
                p_scr[g] = pair_softmax(_mm(cur[:, :PW], expand(cur[:, PW:]), _NT))
                cur = nxt
            out = None
            for g in range(NP + _LAG):
                if g + 1 < NP:
                    nxt = _mm(h, _unpack(wv[g + 1]))
                if g < NP:
                    o_scr[g] = _mm(p_scr[g], expand(full(cur, g, 2 * PW, 3 * PW)))
                    cur = nxt
                if g >= _LAG:
                    part = _mm(o_scr[g - _LAG], _unpack(wo[g - _LAG]))
                    out = part if out is None else out + part
            xs[s] = xs[s] + out[M:]
            return out[:M]

        def a_steps(lo, hi, light, unroll):
            def body(i, carry):
                if light:
                    pl.when(i == 1)(rest_cp.wait)
                    segs = pl.ds(jnp.minimum((i + 1) * SPI, NSEG - SPI), SPI)
                    xs[segs] = xio[segs].astype(_F32)
                mem = mem_scr[...]
                for u in range(unroll):
                    mem = a_step(i * unroll + u, mem, light)
                mem_scr[...] = mem
                return carry

            lax.fori_loop(lo // unroll, hi // unroll, body, 0)

        def layer_a(n_light):
            xn[0] = _layernorm(xs[0])
            mem_scr[...] = mem0_ref[...].astype(_F32)
            with jax.named_scope("alight"):
                a_steps(0, n_light, True, _UNROLL_LIGHT)
            with jax.named_scope("aloop"):
                a_steps(n_light, NSEG, False, _UNROLL)
            xb[(S - SEG) // 2:, :] = _pack(_layernorm(xs[NSEG - 1]))

        def b_pass1(c, carry):
            xc = _unpack(xb[xb_rows(c * SPC, SPC), :])
            ones = jnp.ones((_SUB, _CHUNK), _F32)

            def project(part, b):
                return _mm(_unpack(bw[part, b * BLK // 2:(b + 1) * BLK // 2, :]), xc, _NT)

            def groups(t):
                return [t[i * GR:(i + 1) * GR] for i in range(BLK // GR)]

            phik, vs = [], []
            for b in range(D // BLK):
                phik += [feature_map(p).astype(_BF) for p in groups(project(1, b))]
            for b in range(D // BLK):
                vs += groups(project(2, b))
            for b in range(D // BLK):
                for i, p in enumerate(groups(project(0, b))):
                    phiq[c, b * (BLK // GR) + i] = _pack(feature_map(p))
            for g in range(NG):
                kv_acc[g] = kv_acc[g] + _mm(jnp.concatenate([vs[g], ones], axis=0), phik[g], _NT)
            return carry

        def out_cp(c):
            segs = pl.ds(c * SPC, SPC)
            return pltpu.make_async_copy(xio.at[segs], out_hbm.at[segs], out_sem.at[c])

        def b_attend(c):
            first = _iota((_SUB, _CHUNK), 0) < _SUB // 2
            outs = []
            for g in range(NG):
                nd = _mm(kv_acc[g], _unpack(phiq[c, g]))
                mixed = 1.0 / (nd[GR:] + 1e-06)
                swapped = pltpu.roll(mixed, _SUB // 2, 0)
                for i in range(GR // _SUB):
                    if (i + 1) * _SUB <= FB:
                        inv = jnp.where(first, mixed, swapped)
                    elif i * _SUB >= FB:
                        inv = jnp.where(first, swapped, mixed)
                    else:
                        inv = mixed
                    outs.append(nd[i * _SUB:(i + 1) * _SUB] * inv)
            return _pack(jnp.concatenate(outs, axis=0).T)

        def layer_b(last):
            kv_acc[...] = jnp.zeros(kv_acc.shape, _F32)
            with jax.named_scope("b1"):
                lax.fori_loop(0, NCH, b_pass1, 0, unroll=_UNROLL_B)
            shape = (GR + _SUB, 2 * GR)
            row = _iota(shape, 0)
            second = ((row >= FB) & (row < GR)) | (row >= GR + _SUB // 2)
            same_head = jnp.where(second, 1, 0) == _iota(shape, 1) % 2
            for g in range(NG):
                kv_acc[g] = jnp.where(same_head, kv_acc[g], 0.0)
            with jax.named_scope("b2"):
                ob[...] = b_attend(0)

                def b_pass2(c, carry):
                    o = _unpack(ob[...])
                    ob[...] = b_attend(jnp.minimum(c + 1, NCH - 1))
                    segs = pl.ds(c * SPC, SPC)
                    y = xs[segs] + _mm(o, _unpack(bwo[...])).reshape(SPC, SEG, D)
                    xs[segs] = y
                    xio[segs] = y.astype(_BF)
                    pl.when(last)(out_cp(c).start)
                    return carry

                lax.fori_loop(0, NCH, b_pass2, 0)

        def layer_pair(i, carry):
            layer_a(jnp.where(i == 0, _LIGHT, 0))
            with jax.named_scope("prep"):
                pl.when(i == 0)(prep_b_weights)
            layer_b(i == 1)
            return carry

        lax.fori_loop(0, 2, layer_pair, 0)
        for c in range(NCH):
            out_cp(c).wait()

    scratch = [
        pltpu.VMEM((NP, D // 2, 2 * PW), _U32),
        pltpu.VMEM((NP, D // 2, PW), _U32),
        pltpu.VMEM((NP, PW // 2, D), _U32),
        pltpu.VMEM((_RING, 4, PW, D), _BF),
        pltpu.VMEM((_LIGHT, _SUB, D), _BF),
        pltpu.VMEM((_LIGHT * _SUB // 2, D), _U32),
        pltpu.VMEM((NP, _LIGHT * _SUB, 3 * PW), _F32),
        pltpu.VMEM((NSEG, SEG, D), _BF),
        pltpu.VMEM((NSEG, SEG, D), _F32),
        pltpu.VMEM((S // 2, D), _U32),
        pltpu.VMEM((2, SEG, D), _F32),
        pltpu.VMEM((M, D), _F32),
        pltpu.VMEM((NP, L, 2 * L), _F32),
        pltpu.VMEM((NP, L, PW), _F32),
        pltpu.VMEM((D, 3 * D), _BF),
        pltpu.VMEM((D, D), _BF),
        pltpu.VMEM((3, D // 2, D), _U32),
        pltpu.VMEM((D // 2, D), _U32),
        pltpu.VMEM((NCH, NG, GR, _CHUNK), _U32),
        pltpu.VMEM((NG, GR + _SUB, 2 * GR), _F32),
        pltpu.VMEM((_CHUNK // 2, D), _U32),
        pltpu.SemaphoreType.DMA((_RING, 4)),
        pltpu.SemaphoreType.DMA((5,)),
        pltpu.SemaphoreType.DMA((NCH,)),
    ]
    return kernel, scratch


def pallas_interleave_layers__memory_aug_recurrent_mem_tr__linear_kernel_hedgehog__prompt_kernel(
    A_x, A_mem0, A_Wq, A_Wk, A_Wv, A_Wo, A_seg_len, B_x, B_wqkv, B_w_phi, B_wo,
):
    del B_x
    _, S, D = A_x.shape
    M = A_mem0.shape[1]
    _, H, DH = A_Wq.shape
    HB = B_w_phi.shape[0]
    SEG = int(A_seg_len)
    kernel, scratch = _make_kernel(S, D, M, SEG, H, DH, HB)

    def head_major(w):
        return jnp.transpose(w, (1, 2, 0)).reshape(H * DH, D)

    hbm = pl.BlockSpec(memory_space=pl.ANY)
    vmem = pl.BlockSpec(memory_space=pltpu.VMEM)
    out = pl.pallas_call(
        kernel,
        out_shape=jax.ShapeDtypeStruct((S // SEG, SEG, D), A_x.dtype),
        in_specs=[hbm, vmem, hbm, hbm, hbm, hbm, hbm, vmem, hbm],
        out_specs=hbm,
        scratch_shapes=scratch,
        compiler_params=pltpu.CompilerParams(vmem_limit_bytes=120 * 1024 * 1024, disable_bounds_checks=True),
    )(
        A_x.reshape(S // SEG, SEG, D),
        A_mem0.reshape(M, D),
        head_major(A_Wq),
        head_major(A_Wk),
        head_major(A_Wv),
        A_Wo.reshape(H * DH, D),
        B_wqkv,
        jnp.transpose(B_w_phi, (1, 2, 0)),
        B_wo,
    )
    return out.reshape(A_x.shape)
```

```python
import jax
import jax.numpy as jnp
from jax import lax
import jax.experimental.pallas as pl
import jax.experimental.pallas.tpu as pltpu

_BF = jnp.bfloat16
_F32 = jnp.float32
_U32 = jnp.uint32
_NN = (((1,), (0,)), ((), ()))
_NT = (((1,), (1,)), ((), ()))
_LANES = 128
_SUB = 8
_EPS = 1e-05
_LOG2E = 1.4426950408889634

_RING = 4
_CHUNK = 256
_LIGHT = 40
_UNROLL = 2
_UNROLL_LIGHT = 2
_LAG = 2
_UNROLL_B = 2


def _mm(a, b, dims=_NN):
    return lax.dot_general(a, b, dims, preferred_element_type=_F32)


def _iota(shape, dim):
    return lax.broadcasted_iota(jnp.int32, shape, dim)


def _pack(x):
    return pltpu.bitcast(x.astype(_BF), _U32)


def _unpack(x):
    return pltpu.bitcast(x, _BF)


def _layernorm(x):
    m = jnp.mean(x, axis=-1, keepdims=True)
    c = x - m
    v = jnp.mean(c * c, axis=-1, keepdims=True)
    return c * lax.rsqrt(v + _EPS)


def _make_kernel(S, D, M, SEG, H, DH, HB):
    L = M + SEG
    NSEG = S // SEG
    NP = H // 2
    PW = 2 * DH
    FB = D // HB
    NG = HB // 2
    GR = 2 * FB
    BLK = 4 * GR
    NCH = S // _CHUNK
    SPC = _CHUNK // SEG
    SPI = 2 * _UNROLL_LIGHT
    KEEP = SEG - _SUB
    scale = DH ** (-0.5)
    split_tile = DH // _LANES
    split_lane = DH % _LANES

    def expand(t):
        zero = jnp.zeros((L, _LANES), _F32)
        in_a = _iota((L, _LANES), 1) < split_lane
        top, bot = [], []
        for j in range(PW // _LANES):
            blk = t[:, j * _LANES:(j + 1) * _LANES]
            if j < split_tile:
                top.append(blk)
                bot.append(zero)
            elif j == split_tile:
                top.append(jnp.where(in_a, blk, 0.0))
                bot.append(jnp.where(in_a, 0.0, blk))
            else:
                top.append(zero)
                bot.append(blk)
        both = [jnp.concatenate(top, axis=1), jnp.concatenate(bot, axis=1)]
        return jnp.concatenate(both, axis=0).astype(_BF)

    def pair_softmax(s):
        row = _iota((L, 2 * L), 0)
        col = _iota((L, 2 * L), 1)
        is_a = col < L
        key = jnp.where(is_a, col, col - L)
        s = jnp.where((row < M) | (row >= key), s * scale, -1000000000.0)
        max_a = jnp.max(jnp.where(is_a, s, -jnp.inf), axis=1, keepdims=True)
        max_b = jnp.max(jnp.where(is_a, -jnp.inf, s), axis=1, keepdims=True)
        e = jnp.exp(s - jnp.where(is_a, max_a, max_b))
        sum_a = jnp.sum(jnp.where(is_a, e, 0.0), axis=1, keepdims=True)
        sum_b = jnp.sum(jnp.where(is_a, 0.0, e), axis=1, keepdims=True)
        return e / jnp.where(is_a, sum_a, sum_b)

    def over_features(op, rows):
        r = rows[0]
        for t in rows[1:]:
            r = op(r, t)
        r = op(r, pltpu.roll(r, 4, 0))
        return op(r, pltpu.roll(r, 2, 0))

    def feature_map(p):
        rows = [p[i * _SUB:(i + 1) * _SUB] for i in range(GR // _SUB)]
        hi = over_features(jnp.maximum, rows)
        lo = over_features(jnp.minimum, rows)
        out = []
        for es in ([jnp.exp2(r - hi) for r in rows], [jnp.exp2(lo - r) for r in rows]):
            inv = 1.0 / over_features(jnp.add, es)
            out += [e * inv for e in es]
        return jnp.concatenate(out, axis=0)

    def kernel(x_hbm, mem0_hbm, wq_hbm, wk_hbm, wv_hbm, wo_hbm, bqkv_hbm, phi_hbm, bwo_hbm,
               out_hbm,
               wqk, wv, wo, stage, xtail, xpre, pre, xio, xs, xb, xn, mem_scr, p_scr, o_scr,
               mem0_ref, phi_ref, bqkv_in, bwo_in, bw, bwo, phiq, kv_acc, ob,
               stage_sem, misc_sem, out_sem):

        tail_cp = pltpu.make_async_copy(
            x_hbm.at[pl.ds(0, _LIGHT), pl.ds(KEEP, _SUB)], xtail, misc_sem.at[0])
        mem0_cp = pltpu.make_async_copy(mem0_hbm, mem0_ref, misc_sem.at[5])
        phi_cp = pltpu.make_async_copy(phi_hbm, phi_ref, misc_sem.at[6])
        head, rest = pl.ds(0, 2 * SPI), pl.ds(2 * SPI, NSEG - 2 * SPI)
        head_cp = pltpu.make_async_copy(x_hbm.at[head], xio.at[head], misc_sem.at[3])
        rest_cp = pltpu.make_async_copy(x_hbm.at[rest], xio.at[rest], misc_sem.at[4])
        bqkv_cp = pltpu.make_async_copy(bqkv_hbm, bqkv_in, misc_sem.at[1])
        bwo_cp = pltpu.make_async_copy(bwo_hbm, bwo_in, misc_sem.at[2])

        def stage_cps(g, slot):
            rows = pl.ds(pl.multiple_of(g * PW, PW), PW)
            return [pltpu.make_async_copy(src.at[rows], stage.at[slot, i], stage_sem.at[slot, i])
                    for i, src in enumerate((wq_hbm, wk_hbm, wv_hbm, wo_hbm))]

        tail_cp.start()
        for cp in stage_cps(0, 0):
            cp.start()
        with jax.named_scope("tailwait"):
            tail_cp.wait()
        xpre[...] = _pack(_layernorm(xtail[...].astype(_F32).reshape(_LIGHT * _SUB, D)))
        for g in range(1, _RING - 1):
            for cp in stage_cps(g, g):
                cp.start()

        def load_pair(g, carry):
            nxt = g + _RING - 1

            @pl.when(nxt < NP)
            def _():
                for cp in stage_cps(nxt, nxt % _RING):
                    cp.start()

            @pl.when(nxt == NP)
            def _():
                head_cp.start()
                mem0_cp.start()

            slot = g % _RING
            for cp in stage_cps(g, slot):
                cp.wait()
            wo[g] = _pack(stage[slot, 3])
            lhs = _unpack(xpre[...])
            pre[g, :, :_LANES] = _mm(lhs, stage[slot, 0, :_LANES], _NT)
            w = stage[slot, 0].T
            wqk[g, :, :PW] = _pack(w)
            pre[g, :, _LANES:PW] = _mm(lhs, w[:, _LANES:])
            w = stage[slot, 1].T
            wqk[g, :, PW:] = _pack(w)
            pre[g, :, PW:2 * PW] = _mm(lhs, w)
            w = stage[slot, 2].T
            wv[g] = _pack(w)
            pre[g, :, 2 * PW:] = _mm(lhs, w)
            return carry

        with jax.named_scope("load"):
            lax.fori_loop(0, NP, load_pair, 0)
        rest_cp.start()
        bqkv_cp.start()
        bwo_cp.start()
        phi_cp.start()
        head_cp.wait()
        mem0_cp.wait()
        xs[0:SPI] = xio[0:SPI].astype(_F32)

        def prep_b_weights():
            bqkv_cp.wait()
            bwo_cp.wait()
            phi_cp.wait()
            head = _iota((HB, D), 0)
            col = _iota((HB, D), 1)
            t = None
            for d in range(FB):
                sel = jnp.where(col == head * FB + d, 1.0, 0.0).astype(_BF)
                part = _mm(phi_ref[d].astype(_F32), sel)
                t = part if t is None else t + part
            dup = jnp.where(_iota((GR, FB), 0) // 2 == _iota((GR, FB), 1), 1.0, 0.0)
            t = _mm(dup, t.astype(_BF))
            off = _iota((GR, D), 1) - (_iota((GR, D), 0) % 2) * FB
            phi_t = [jnp.where((off >= g * GR) & (off < g * GR + FB), t, 0.0) for g in range(NG)]
            bw[2] = _pack(bqkv_in[:, 2 * D:].T)
            bwo[...] = _pack(bwo_in[...])
            for part in range(2):
                acc = [None] * NG
                for j in range(D // _LANES):
                    lo, hi = j * _LANES, (j + 1) * _LANES
                    gs = range(lo // GR, (hi - 1) // GR + 1)
                    lhs = jnp.concatenate([phi_t[g][:, lo:hi] for g in gs], axis=0)
                    r = _mm(lhs, bqkv_in[:, part * D + lo:part * D + hi], _NT)
                    for i, g in enumerate(gs):
                        piece = r[i * GR:(i + 1) * GR]
                        acc[g] = piece if acc[g] is None else acc[g] + piece
                bw[part] = _pack(jnp.concatenate(acc, axis=0) * _LOG2E)

        def xb_rows(s, n):
            return pl.ds(pl.multiple_of(s * (SEG // 2), SEG // 2), n * (SEG // 2))

        def a_step(s, mem, light):
            if light:
                h = jnp.concatenate([mem, xn[s % 2, :KEEP]], axis=0).astype(_BF)
                tail = pl.ds(pl.multiple_of(s * _SUB, _SUB), _SUB)
                full = lambda r, g, a, b: jnp.concatenate([r, pre[g, tail, a:b]], axis=0)
            else:
                h = jnp.concatenate([mem, xn[s % 2]], axis=0)
                full = lambda r, g, a, b: r
            xn[(s + 1) % 2] = _layernorm(xs[jnp.minimum(s + 1, NSEG - 1)])
            prev = jnp.maximum(s - 1, 0)
            xb[xb_rows(prev, 1), :] = _pack(_layernorm(xs[prev]))

            cur = None
            for k in range(D // _LANES):
                w = _unpack(wqk[0, k * _LANES // 2:(k + 1) * _LANES // 2, :])
                part = _mm(h[:, k * _LANES:(k + 1) * _LANES], w)
                cur = part if cur is None else cur + part
            for g in range(NP):
                nxt = _mm(h, _unpack(wqk[g + 1] if g + 1 < NP else wv[0]))
                cur = full(cur, g, 0, 2 * PW)
                p_scr[g] = pair_softmax(_mm(cur[:, :PW], expand(cur[:, PW:]), _NT))
                cur = nxt
            out = None
            for g in range(NP + _LAG):
                if g + 1 < NP:
                    nxt = _mm(h, _unpack(wv[g + 1]))
                if g < NP:
                    o_scr[g] = _mm(p_scr[g], expand(full(cur, g, 2 * PW, 3 * PW)))
                    cur = nxt
                if g >= _LAG:
                    part = _mm(o_scr[g - _LAG], _unpack(wo[g - _LAG]))
                    out = part if out is None else out + part
            xs[s] = xs[s] + out[M:]
            return out[:M]

        def a_steps(lo, hi, light, unroll):
            def body(i, carry):
                if light:
                    pl.when(i == 1)(rest_cp.wait)
                mem = mem_scr[...]
                for u in range(unroll):
                    mem = a_step(i * unroll + u, mem, light)
                    if light and u == 0:
                        segs = pl.ds(jnp.minimum((i + 1) * SPI, NSEG - SPI), SPI)
                        xs[segs] = xio[segs].astype(_F32)
                mem_scr[...] = mem
                return carry

            lax.fori_loop(lo // unroll, hi // unroll, body, 0)

        def layer_a(n_light):
            xn[0] = _layernorm(xs[0])
            mem_scr[...] = mem0_ref[...].astype(_F32)
            with jax.named_scope("alight"):
                a_steps(0, n_light, True, _UNROLL_LIGHT)
            with jax.named_scope("aloop"):
                a_steps(n_light, NSEG, False, _UNROLL)
            xb[(S - SEG) // 2:, :] = _pack(_layernorm(xs[NSEG - 1]))

        def b_pass1(c, carry):
            xc = _unpack(xb[xb_rows(c * SPC, SPC), :])
            ones = jnp.ones((_SUB, _CHUNK), _F32)

            def project(part, b):
                return _mm(_unpack(bw[part, b * BLK // 2:(b + 1) * BLK // 2, :]), xc, _NT)

            def groups(t):
                return [t[i * GR:(i + 1) * GR] for i in range(BLK // GR)]

            phik, vs = [], []
            for b in range(D // BLK):
                phik += [feature_map(p).astype(_BF) for p in groups(project(1, b))]
            for b in range(D // BLK):
                vs += groups(project(2, b))
            for b in range(D // BLK):
                for i, p in enumerate(groups(project(0, b))):
                    phiq[c, b * (BLK // GR) + i] = _pack(feature_map(p))
            for g in range(NG):
                kv_acc[g] = kv_acc[g] + _mm(jnp.concatenate([vs[g], ones], axis=0), phik[g], _NT)
            return carry

        def out_cp(c):
            segs = pl.ds(c * SPC, SPC)
            return pltpu.make_async_copy(xio.at[segs], out_hbm.at[segs], out_sem.at[c])

        def b_attend(c):
            first = _iota((_SUB, _CHUNK), 0) < _SUB // 2
            outs = []
            for g in range(NG):
                nd = _mm(kv_acc[g], _unpack(phiq[c, g]))
                mixed = 1.0 / (nd[GR:] + 1e-06)
                swapped = pltpu.roll(mixed, _SUB // 2, 0)
                for i in range(GR // _SUB):
                    if (i + 1) * _SUB <= FB:
                        inv = jnp.where(first, mixed, swapped)
                    elif i * _SUB >= FB:
                        inv = jnp.where(first, swapped, mixed)
                    else:
                        inv = mixed
                    outs.append(nd[i * _SUB:(i + 1) * _SUB] * inv)
            return _pack(jnp.concatenate(outs, axis=0).T)

        def layer_b(last):
            kv_acc[...] = jnp.zeros(kv_acc.shape, _F32)
            with jax.named_scope("b1"):
                lax.fori_loop(0, NCH, b_pass1, 0, unroll=_UNROLL_B)
            shape = (GR + _SUB, 2 * GR)
            row = _iota(shape, 0)
            second = ((row >= FB) & (row < GR)) | (row >= GR + _SUB // 2)
            same_head = jnp.where(second, 1, 0) == _iota(shape, 1) % 2
            for g in range(NG):
                kv_acc[g] = jnp.where(same_head, kv_acc[g], 0.0)
            with jax.named_scope("b2"):
                ob[...] = b_attend(0)

                def b_pass2(c, carry):
                    o = _unpack(ob[...])
                    ob[...] = b_attend(jnp.minimum(c + 1, NCH - 1))
                    segs = pl.ds(c * SPC, SPC)
                    y = xs[segs] + _mm(o, _unpack(bwo[...])).reshape(SPC, SEG, D)
                    xs[segs] = y
                    xio[segs] = y.astype(_BF)
                    pl.when(last)(out_cp(c).start)
                    return carry

                lax.fori_loop(0, NCH, b_pass2, 0)

        def layer_pair(i, carry):
            layer_a(jnp.where(i == 0, _LIGHT, 0))
            with jax.named_scope("prep"):
                pl.when(i == 0)(prep_b_weights)
            layer_b(i == 1)
            return carry

        lax.fori_loop(0, 2, layer_pair, 0)
        for c in range(NCH):
            out_cp(c).wait()

    scratch = [
        pltpu.VMEM((NP, D // 2, 2 * PW), _U32),
        pltpu.VMEM((NP, D // 2, PW), _U32),
        pltpu.VMEM((NP, PW // 2, D), _U32),
        pltpu.VMEM((_RING, 4, PW, D), _BF),
        pltpu.VMEM((_LIGHT, _SUB, D), _BF),
        pltpu.VMEM((_LIGHT * _SUB // 2, D), _U32),
        pltpu.VMEM((NP, _LIGHT * _SUB, 3 * PW), _F32),
        pltpu.VMEM((NSEG, SEG, D), _BF),
        pltpu.VMEM((NSEG, SEG, D), _F32),
        pltpu.VMEM((S // 2, D), _U32),
        pltpu.VMEM((2, SEG, D), _F32),
        pltpu.VMEM((M, D), _F32),
        pltpu.VMEM((NP, L, 2 * L), _F32),
        pltpu.VMEM((NP, L, PW), _F32),
        pltpu.VMEM((M, D), _BF),
        pltpu.VMEM((FB, FB, HB), _BF),
        pltpu.VMEM((D, 3 * D), _BF),
        pltpu.VMEM((D, D), _BF),
        pltpu.VMEM((3, D // 2, D), _U32),
        pltpu.VMEM((D // 2, D), _U32),
        pltpu.VMEM((NCH, NG, GR, _CHUNK), _U32),
        pltpu.VMEM((NG, GR + _SUB, 2 * GR), _F32),
        pltpu.VMEM((_CHUNK // 2, D), _U32),
        pltpu.SemaphoreType.DMA((_RING, 4)),
        pltpu.SemaphoreType.DMA((7,)),
        pltpu.SemaphoreType.DMA((NCH,)),
    ]
    return kernel, scratch


def pallas_interleave_layers__memory_aug_recurrent_mem_tr__linear_kernel_hedgehog__prompt_kernel(
    A_x, A_mem0, A_Wq, A_Wk, A_Wv, A_Wo, A_seg_len, B_x, B_wqkv, B_w_phi, B_wo,
):
    del B_x
    _, S, D = A_x.shape
    M = A_mem0.shape[1]
    _, H, DH = A_Wq.shape
    HB = B_w_phi.shape[0]
    SEG = int(A_seg_len)
    kernel, scratch = _make_kernel(S, D, M, SEG, H, DH, HB)

    def head_major(w):
        return jnp.transpose(w, (1, 2, 0)).reshape(H * DH, D)

    hbm = pl.BlockSpec(memory_space=pl.ANY)
    out = pl.pallas_call(
        kernel,
        out_shape=jax.ShapeDtypeStruct((S // SEG, SEG, D), A_x.dtype),
        in_specs=[hbm] * 9,
        out_specs=hbm,
        scratch_shapes=scratch,
        compiler_params=pltpu.CompilerParams(vmem_limit_bytes=120 * 1024 * 1024, disable_bounds_checks=True),
    )(
        A_x.reshape(S // SEG, SEG, D),
        A_mem0.reshape(M, D),
        head_major(A_Wq),
        head_major(A_Wk),
        head_major(A_Wv),
        A_Wo.reshape(H * DH, D),
        B_wqkv,
        jnp.transpose(B_w_phi, (1, 2, 0)),
        B_wo,
    )
    return out.reshape(A_x.shape)
```

```python
import jax
import jax.numpy as jnp
from jax import lax
import jax.experimental.pallas as pl
import jax.experimental.pallas.tpu as pltpu

_BF = jnp.bfloat16
_F32 = jnp.float32
_U32 = jnp.uint32
_NN = (((1,), (0,)), ((), ()))
_NT = (((1,), (1,)), ((), ()))
_LANES = 128
_SUB = 8
_EPS = 1e-05
_LOG2E = 1.4426950408889634

_RING = 4
_CHUNK = 256
_LIGHT = 40
_UNROLL = 2
_UNROLL_LIGHT = 2
_LAG = 2
_UNROLL_B = 2
_LIGHT_ORDER = "qqqoqsqoqvvovp"


def _mm(a, b, dims=_NN):
    return lax.dot_general(a, b, dims, preferred_element_type=_F32)


def _iota(shape, dim):
    return lax.broadcasted_iota(jnp.int32, shape, dim)


def _pack(x):
    return pltpu.bitcast(x.astype(_BF), _U32)


def _unpack(x):
    return pltpu.bitcast(x, _BF)


def _layernorm(x):
    m = jnp.mean(x, axis=-1, keepdims=True)
    c = x - m
    v = jnp.mean(c * c, axis=-1, keepdims=True)
    return c * lax.rsqrt(v + _EPS)


def _make_kernel(S, D, M, SEG, H, DH, HB):
    L = M + SEG
    NSEG = S // SEG
    NP = H // 2
    PW = 2 * DH
    FB = D // HB
    NG = HB // 2
    GR = 2 * FB
    BLK = 4 * GR
    NCH = S // _CHUNK
    SPC = _CHUNK // SEG
    SPI = 2 * _UNROLL_LIGHT
    KEEP = SEG - _SUB
    scale = DH ** (-0.5)
    split_tile = DH // _LANES
    split_lane = DH % _LANES

    def expand(t):
        zero = jnp.zeros((L, _LANES), _F32)
        in_a = _iota((L, _LANES), 1) < split_lane
        top, bot = [], []
        for j in range(PW // _LANES):
            blk = t[:, j * _LANES:(j + 1) * _LANES]
            if j < split_tile:
                top.append(blk)
                bot.append(zero)
            elif j == split_tile:
                top.append(jnp.where(in_a, blk, 0.0))
                bot.append(jnp.where(in_a, 0.0, blk))
            else:
                top.append(zero)
                bot.append(blk)
        both = [jnp.concatenate(top, axis=1), jnp.concatenate(bot, axis=1)]
        return jnp.concatenate(both, axis=0).astype(_BF)

    def pair_softmax(s):
        row = _iota((L, 2 * L), 0)
        col = _iota((L, 2 * L), 1)
        is_a = col < L
        key = jnp.where(is_a, col, col - L)
        s = jnp.where((row < M) | (row >= key), s * scale, -1000000000.0)
        max_a = jnp.max(jnp.where(is_a, s, -jnp.inf), axis=1, keepdims=True)
        max_b = jnp.max(jnp.where(is_a, -jnp.inf, s), axis=1, keepdims=True)
        e = jnp.exp(s - jnp.where(is_a, max_a, max_b))
        sum_a = jnp.sum(jnp.where(is_a, e, 0.0), axis=1, keepdims=True)
        sum_b = jnp.sum(jnp.where(is_a, 0.0, e), axis=1, keepdims=True)
        return e / jnp.where(is_a, sum_a, sum_b)

    def over_features(op, rows):
        r = rows[0]
        for t in rows[1:]:
            r = op(r, t)
        r = op(r, pltpu.roll(r, 4, 0))
        return op(r, pltpu.roll(r, 2, 0))

    def feature_map(p):
        rows = [p[i * _SUB:(i + 1) * _SUB] for i in range(GR // _SUB)]
        hi = over_features(jnp.maximum, rows)
        lo = over_features(jnp.minimum, rows)
        out = []
        for es in ([jnp.exp2(r - hi) for r in rows], [jnp.exp2(lo - r) for r in rows]):
            inv = 1.0 / over_features(jnp.add, es)
            out += [e * inv for e in es]
        return jnp.concatenate(out, axis=0)

    def kernel(x_hbm, mem0_hbm, wq_hbm, wk_hbm, wv_hbm, wo_hbm, bqkv_hbm, phi_hbm, bwo_hbm,
               out_hbm,
               wqk, wv, wo, stage, xtail, xpre, pre, xio, xs, xb, xn, mem_scr, p_scr, o_scr,
               mem0_ref, phi_ref, bqkv_in, bwo_in, bw, bwo, phiq, kv_acc, ob,
               stage_sem, misc_sem, out_sem):

        tail_cp = pltpu.make_async_copy(
            x_hbm.at[pl.ds(0, _LIGHT), pl.ds(KEEP, _SUB)], xtail, misc_sem.at[0])
        mem0_cp = pltpu.make_async_copy(mem0_hbm, mem0_ref, misc_sem.at[5])
        phi_cp = pltpu.make_async_copy(phi_hbm, phi_ref, misc_sem.at[6])
        head, rest = pl.ds(0, 2 * SPI), pl.ds(2 * SPI, NSEG - 2 * SPI)
        head_cp = pltpu.make_async_copy(x_hbm.at[head], xio.at[head], misc_sem.at[3])
        rest_cp = pltpu.make_async_copy(x_hbm.at[rest], xio.at[rest], misc_sem.at[4])
        bqkv_cp = pltpu.make_async_copy(bqkv_hbm, bqkv_in, misc_sem.at[1])
        bwo_cp = pltpu.make_async_copy(bwo_hbm, bwo_in, misc_sem.at[2])

        def stage_cp(src, g, slot, i):
            rows = pl.ds(pl.multiple_of(g * PW, PW), PW)
            return pltpu.make_async_copy(src.at[rows], stage.at[slot, i], stage_sem.at[slot, i])

        def qkv_cps(g):
            return [stage_cp(src, g, g % _RING, i)
                    for i, src in enumerate((wq_hbm, wk_hbm, wv_hbm))]

        def wo_cp(g):
            return stage_cp(wo_hbm, g, (g + 1) % _RING, 3)

        tail_cp.start()
        for cp in qkv_cps(0):
            cp.start()
        with jax.named_scope("tailwait"):
            tail_cp.wait()
        xpre[...] = _pack(_layernorm(xtail[...].astype(_F32).reshape(_LIGHT * _SUB, D)))
        for g in range(1, _RING - 1):
            for cp in qkv_cps(g) + [wo_cp(g - 1)]:
                cp.start()

        def load_pair(g, carry):
            nxt = g + _RING - 1

            @pl.when(nxt < NP)
            def _():
                for cp in qkv_cps(nxt):
                    cp.start()

            @pl.when(nxt <= NP)
            def _():
                wo_cp(nxt - 1).start()

            @pl.when(nxt == NP)
            def _():
                head_cp.start()
                mem0_cp.start()

            slot = g % _RING
            prev = jnp.maximum(g - 1, 0)
            for cp in qkv_cps(g):
                cp.wait()
            pl.when(g > 0)(wo_cp(prev).wait)
            wo[prev] = _pack(stage[slot, jnp.where(g > 0, 3, 0)])
            lhs = _unpack(xpre[...])
            pre[g, :, :_LANES] = _mm(lhs, stage[slot, 0, :_LANES], _NT)
            w = stage[slot, 0].T
            wqk[g, :, :PW] = _pack(w)
            pre[g, :, _LANES:PW] = _mm(lhs, w[:, _LANES:])
            w = stage[slot, 1].T
            wqk[g, :, PW:] = _pack(w)
            pre[g, :, PW:2 * PW] = _mm(lhs, w)
            w = stage[slot, 2].T
            wv[g] = _pack(w)
            pre[g, :, 2 * PW:] = _mm(lhs, w)
            return carry

        with jax.named_scope("load"):
            lax.fori_loop(0, NP, load_pair, 0)
        rest_cp.start()
        bqkv_cp.start()
        bwo_cp.start()
        phi_cp.start()
        wo_cp(NP - 1).wait()
        wo[NP - 1] = _pack(stage[NP % _RING, 3])
        head_cp.wait()
        mem0_cp.wait()
        xs[0:SPI] = xio[0:SPI].astype(_F32)

        def prep_b_weights():
            bqkv_cp.wait()
            bwo_cp.wait()
            phi_cp.wait()
            head = _iota((HB, D), 0)
            col = _iota((HB, D), 1)
            t = None
            for d in range(FB):
                sel = jnp.where(col == head * FB + d, 1.0, 0.0).astype(_BF)
                part = _mm(phi_ref[d].astype(_F32), sel)
                t = part if t is None else t + part
            dup = jnp.where(_iota((GR, FB), 0) // 2 == _iota((GR, FB), 1), 1.0, 0.0)
            t = _mm(dup, t.astype(_BF))
            off = _iota((GR, D), 1) - (_iota((GR, D), 0) % 2) * FB
            phi_t = [jnp.where((off >= g * GR) & (off < g * GR + FB), t, 0.0) for g in range(NG)]
            bw[2] = _pack(bqkv_in[:, 2 * D:].T)
            bwo[...] = _pack(bwo_in[...])
            for part in range(2):
                acc = [None] * NG
                for j in range(D // _LANES):
                    lo, hi = j * _LANES, (j + 1) * _LANES
                    gs = range(lo // GR, (hi - 1) // GR + 1)
                    lhs = jnp.concatenate([phi_t[g][:, lo:hi] for g in gs], axis=0)
                    r = _mm(lhs, bqkv_in[:, part * D + lo:part * D + hi], _NT)
                    for i, g in enumerate(gs):
                        piece = r[i * GR:(i + 1) * GR]
                        acc[g] = piece if acc[g] is None else acc[g] + piece
                bw[part] = _pack(jnp.concatenate(acc, axis=0) * _LOG2E)

        def xb_rows(s, n):
            return pl.ds(pl.multiple_of(s * (SEG // 2), SEG // 2), n * (SEG // 2))

        def tile(i):
            return slice(i * _LANES, (i + 1) * _LANES)

        def packed_tile(i):
            return slice(i * _LANES // 2, (i + 1) * _LANES // 2)

        def add(acc, x):
            return x if acc is None else acc + x

        def a_step(s, mem, light):
            h = jnp.concatenate([mem, xn[s % 2, :KEEP if light else SEG]], axis=0)
            if light:
                h = h.astype(_BF)
            xn[(s + 1) % 2] = _layernorm(xs[jnp.minimum(s + 1, NSEG - 1)])
            prev = jnp.maximum(s - 1, 0)
            xb[xb_rows(prev, 1), :] = _pack(_layernorm(xs[prev]))
            qk = None
            for k in range(D // _LANES):
                qk = add(qk, _mm(h[:, tile(k)], _unpack(wqk[0, packed_tile(k), :])))
            out = a_light(s, h, qk) if light else a_full(h, qk)
            xs[s] = xs[s] + out[M:]
            return out[:M]

        def scores(g, qk):
            p_scr[g] = pair_softmax(_mm(qk[:, :PW], expand(qk[:, PW:]), _NT))

        def a_full(h, cur):
            for g in range(NP):
                nxt = _mm(h, _unpack(wqk[g + 1] if g + 1 < NP else wv[0]))
                scores(g, cur)
                cur = nxt
            out = None
            for g in range(NP + _LAG):
                if g + 1 < NP:
                    nxt = _mm(h, _unpack(wv[g + 1]))
                if g < NP:
                    o_scr[g] = _mm(p_scr[g], expand(cur))
                    cur = nxt
                if g >= _LAG:
                    out = add(out, _mm(o_scr[g - _LAG], _unpack(wo[g - _LAG])))
            return out

        def a_light(s, h, qk):
            tail = pl.ds(pl.multiple_of(s * _SUB, _SUB), _SUB)
            out = v = None
            for t in range(1, NP + _LAG + 2):
                qk_new, v_new, n_out = [], [], 0
                g = t - 2 - _LAG
                for op in _LIGHT_ORDER:
                    if op == "q" and t < NP:
                        qk_new.append(_mm(h, _unpack(wqk[t, :, tile(len(qk_new))])))
                    elif op == "v" and t - 1 < NP:
                        v_new.append(_mm(h, _unpack(wv[t - 1, :, tile(len(v_new))])))
                    elif op == "s" and t - 1 < NP:
                        scores(t - 1, jnp.concatenate([qk, pre[t - 1, tail, :2 * PW]], axis=0))
                    elif op == "p" and 0 <= t - 2 < NP:
                        full = jnp.concatenate([v, pre[t - 2, tail, 2 * PW:]], axis=0)
                        o_scr[t - 2] = _mm(p_scr[t - 2], expand(full))
                    elif op == "o":
                        if 0 <= g < NP - 1:
                            w = _unpack(wo[g, packed_tile(n_out), :])
                            out = add(out, _mm(o_scr[g, :, tile(n_out)], w))
                        elif g == NP - 1 and n_out == 0:
                            out = out + _mm(o_scr[g], _unpack(wo[g]))
                        n_out += 1
                if qk_new:
                    qk = jnp.concatenate(qk_new, axis=1)
                if v_new:
                    v = jnp.concatenate(v_new, axis=1)
            return out

        def a_steps(lo, hi, light, unroll):
            def body(i, carry):
                if light:
                    pl.when(i == 1)(rest_cp.wait)
                mem = mem_scr[...]
                for u in range(unroll):
                    mem = a_step(i * unroll + u, mem, light)
                    if light and u == 0:
                        segs = pl.ds(jnp.minimum((i + 1) * SPI, NSEG - SPI), SPI)
                        xs[segs] = xio[segs].astype(_F32)
                mem_scr[...] = mem
                return carry

            lax.fori_loop(lo // unroll, hi // unroll, body, 0)

        def layer_a(n_light):
            xn[0] = _layernorm(xs[0])
            mem_scr[...] = mem0_ref[...].astype(_F32)
            with jax.named_scope("alight"):
                a_steps(0, n_light, True, _UNROLL_LIGHT)
            with jax.named_scope("aloop"):
                a_steps(n_light, NSEG, False, _UNROLL)
            xb[(S - SEG) // 2:, :] = _pack(_layernorm(xs[NSEG - 1]))

        def b_pass1(c, carry):
            xc = _unpack(xb[xb_rows(c * SPC, SPC), :])
            ones = jnp.ones((_SUB, _CHUNK), _F32)

            def project(part, b):
                return _mm(_unpack(bw[part, b * BLK // 2:(b + 1) * BLK // 2, :]), xc, _NT)

            def groups(t):
                return [t[i * GR:(i + 1) * GR] for i in range(BLK // GR)]

            phik, vs = [], []
            for b in range(D // BLK):
                phik += [feature_map(p).astype(_BF) for p in groups(project(1, b))]
            for b in range(D // BLK):
                vs += groups(project(2, b))
            for b in range(D // BLK):
                for i, p in enumerate(groups(project(0, b))):
                    phiq[c, b * (BLK // GR) + i] = _pack(feature_map(p))
            for g in range(NG):
                kv_acc[g] = kv_acc[g] + _mm(jnp.concatenate([vs[g], ones], axis=0), phik[g], _NT)
            return carry

        def out_cp(c):
            segs = pl.ds(c * SPC, SPC)
            return pltpu.make_async_copy(xio.at[segs], out_hbm.at[segs], out_sem.at[c])

        def b_attend(c):
            first = _iota((_SUB, _CHUNK), 0) < _SUB // 2
            outs = []
            for g in range(NG):
                nd = _mm(kv_acc[g], _unpack(phiq[c, g]))
                mixed = 1.0 / (nd[GR:] + 1e-06)
                swapped = pltpu.roll(mixed, _SUB // 2, 0)
                for i in range(GR // _SUB):
                    if (i + 1) * _SUB <= FB:
                        inv = jnp.where(first, mixed, swapped)
                    elif i * _SUB >= FB:
                        inv = jnp.where(first, swapped, mixed)
                    else:
                        inv = mixed
                    outs.append(nd[i * _SUB:(i + 1) * _SUB] * inv)
            return _pack(jnp.concatenate(outs, axis=0).T)

        def layer_b(last):
            kv_acc[...] = jnp.zeros(kv_acc.shape, _F32)
            with jax.named_scope("b1"):
                lax.fori_loop(0, NCH, b_pass1, 0, unroll=_UNROLL_B)
            shape = (GR + _SUB, 2 * GR)
            row = _iota(shape, 0)
            second = ((row >= FB) & (row < GR)) | (row >= GR + _SUB // 2)
            same_head = jnp.where(second, 1, 0) == _iota(shape, 1) % 2
            for g in range(NG):
                kv_acc[g] = jnp.where(same_head, kv_acc[g], 0.0)
            with jax.named_scope("b2"):
                ob[...] = b_attend(0)

                def b_pass2(c, carry):
                    o = _unpack(ob[...])
                    ob[...] = b_attend(jnp.minimum(c + 1, NCH - 1))
                    segs = pl.ds(c * SPC, SPC)
                    y = xs[segs] + _mm(o, _unpack(bwo[...])).reshape(SPC, SEG, D)
                    xs[segs] = y
                    xio[segs] = y.astype(_BF)
                    pl.when(last)(out_cp(c).start)
                    return carry

                lax.fori_loop(0, NCH, b_pass2, 0, unroll=_UNROLL_B)

        def layer_pair(i, carry):
            layer_a(jnp.where(i == 0, _LIGHT, 0))
            with jax.named_scope("prep"):
                pl.when(i == 0)(prep_b_weights)
            layer_b(i == 1)
            return carry

        lax.fori_loop(0, 2, layer_pair, 0)
        for c in range(NCH):
            out_cp(c).wait()

    scratch = [
        pltpu.VMEM((NP, D // 2, 2 * PW), _U32),
        pltpu.VMEM((NP, D // 2, PW), _U32),
        pltpu.VMEM((NP, PW // 2, D), _U32),
        pltpu.VMEM((_RING, 4, PW, D), _BF),
        pltpu.VMEM((_LIGHT, _SUB, D), _BF),
        pltpu.VMEM((_LIGHT * _SUB // 2, D), _U32),
        pltpu.VMEM((NP, _LIGHT * _SUB, 3 * PW), _F32),
        pltpu.VMEM((NSEG, SEG, D), _BF),
        pltpu.VMEM((NSEG, SEG, D), _F32),
        pltpu.VMEM((S // 2, D), _U32),
        pltpu.VMEM((2, SEG, D), _F32),
        pltpu.VMEM((M, D), _F32),
        pltpu.VMEM((NP, L, 2 * L), _F32),
        pltpu.VMEM((NP, L, PW), _F32),
        pltpu.VMEM((M, D), _BF),
        pltpu.VMEM((FB, FB, HB), _BF),
        pltpu.VMEM((D, 3 * D), _BF),
        pltpu.VMEM((D, D), _BF),
        pltpu.VMEM((3, D // 2, D), _U32),
        pltpu.VMEM((D // 2, D), _U32),
        pltpu.VMEM((NCH, NG, GR, _CHUNK), _U32),
        pltpu.VMEM((NG, GR + _SUB, 2 * GR), _F32),
        pltpu.VMEM((_CHUNK // 2, D), _U32),
        pltpu.SemaphoreType.DMA((_RING, 4)),
        pltpu.SemaphoreType.DMA((7,)),
        pltpu.SemaphoreType.DMA((NCH,)),
    ]
    return kernel, scratch


def pallas_interleave_layers__memory_aug_recurrent_mem_tr__linear_kernel_hedgehog__prompt_kernel(
    A_x, A_mem0, A_Wq, A_Wk, A_Wv, A_Wo, A_seg_len, B_x, B_wqkv, B_w_phi, B_wo,
):
    del B_x
    _, S, D = A_x.shape
    M = A_mem0.shape[1]
    _, H, DH = A_Wq.shape
    HB = B_w_phi.shape[0]
    SEG = int(A_seg_len)
    kernel, scratch = _make_kernel(S, D, M, SEG, H, DH, HB)

    def head_major(w):
        return jnp.transpose(w, (1, 2, 0)).reshape(H * DH, D)

    hbm = pl.BlockSpec(memory_space=pl.ANY)
    out = pl.pallas_call(
        kernel,
        out_shape=jax.ShapeDtypeStruct((S // SEG, SEG, D), A_x.dtype),
        in_specs=[hbm] * 9,
        out_specs=hbm,
        scratch_shapes=scratch,
        compiler_params=pltpu.CompilerParams(vmem_limit_bytes=120 * 1024 * 1024, disable_bounds_checks=True),
    )(
        A_x.reshape(S // SEG, SEG, D),
        A_mem0.reshape(M, D),
        head_major(A_Wq),
        head_major(A_Wk),
        head_major(A_Wv),
        A_Wo.reshape(H * DH, D),
        B_wqkv,
        jnp.transpose(B_w_phi, (1, 2, 0)),
        B_wo,
    )
    return out.reshape(A_x.shape)
```

```python
import jax
import jax.numpy as jnp
from jax import lax
import jax.experimental.pallas as pl
import jax.experimental.pallas.tpu as pltpu

_BF = jnp.bfloat16
_F32 = jnp.float32
_U32 = jnp.uint32
_NN = (((1,), (0,)), ((), ()))
_NT = (((1,), (1,)), ((), ()))
_LANES = 128
_SUB = 8
_EPS = 1e-05
_LOG2E = 1.4426950408889634

_RING = 4
_CHUNK = 256
_LIGHT = 40
_UNROLL = 2
_UNROLL_LIGHT = 2
_LAG = 2
_UNROLL_B = 2
_LIGHT_ORDER = "qqqoqsqoqvvovp"


def _mm(a, b, dims=_NN):
    return lax.dot_general(a, b, dims, preferred_element_type=_F32)


def _add(acc, x):
    return x if acc is None else acc + x


def _iota(shape, dim):
    return lax.broadcasted_iota(jnp.int32, shape, dim)


def _pack(x):
    return pltpu.bitcast(x.astype(_BF), _U32)


def _unpack(x):
    return pltpu.bitcast(x, _BF)


def _layernorm(x):
    m = jnp.mean(x, axis=-1, keepdims=True)
    c = x - m
    v = jnp.mean(c * c, axis=-1, keepdims=True)
    return c * lax.rsqrt(v + _EPS)


def _make_kernel(S, D, M, SEG, H, DH, HB):
    L = M + SEG
    NSEG = S // SEG
    NP = H // 2
    PW = 2 * DH
    FB = D // HB
    NG = HB // 2
    GR = 2 * FB
    BLK = 4 * GR
    NCH = S // _CHUNK
    SPC = _CHUNK // SEG
    SPI = 2 * _UNROLL_LIGHT
    KEEP = SEG - _SUB
    scale = DH ** (-0.5)
    split_tile = DH // _LANES
    split_lane = DH % _LANES

    def expand(t):
        zero = jnp.zeros((L, _LANES), _F32)
        in_a = _iota((L, _LANES), 1) < split_lane
        top, bot = [], []
        for j in range(PW // _LANES):
            blk = t[:, j * _LANES:(j + 1) * _LANES]
            if j < split_tile:
                top.append(blk)
                bot.append(zero)
            elif j == split_tile:
                top.append(jnp.where(in_a, blk, 0.0))
                bot.append(jnp.where(in_a, 0.0, blk))
            else:
                top.append(zero)
                bot.append(blk)
        both = [jnp.concatenate(top, axis=1), jnp.concatenate(bot, axis=1)]
        return jnp.concatenate(both, axis=0).astype(_BF)

    def pair_softmax(s):
        row = _iota((L, 2 * L), 0)
        col = _iota((L, 2 * L), 1)
        is_a = col < L
        key = jnp.where(is_a, col, col - L)
        s = jnp.where((row < M) | (row >= key), s * scale, -1000000000.0)
        max_a = jnp.max(jnp.where(is_a, s, -jnp.inf), axis=1, keepdims=True)
        max_b = jnp.max(jnp.where(is_a, -jnp.inf, s), axis=1, keepdims=True)
        e = jnp.exp(s - jnp.where(is_a, max_a, max_b))
        sum_a = jnp.sum(jnp.where(is_a, e, 0.0), axis=1, keepdims=True)
        sum_b = jnp.sum(jnp.where(is_a, 0.0, e), axis=1, keepdims=True)
        return e / jnp.where(is_a, sum_a, sum_b)

    def over_features(op, rows):
        r = rows[0]
        for t in rows[1:]:
            r = op(r, t)
        r = op(r, pltpu.roll(r, 4, 0))
        return op(r, pltpu.roll(r, 2, 0))

    def feature_map(p):
        rows = [p[i * _SUB:(i + 1) * _SUB] for i in range(GR // _SUB)]
        hi = over_features(jnp.maximum, rows)
        lo = over_features(jnp.minimum, rows)
        out = []
        for es in ([jnp.exp2(r - hi) for r in rows], [jnp.exp2(lo - r) for r in rows]):
            inv = 1.0 / over_features(jnp.add, es)
            out += [e * inv for e in es]
        return jnp.concatenate(out, axis=0)

    def kernel(x_hbm, mem0_hbm, wq_hbm, wk_hbm, wv_hbm, wo_hbm, bqkv_hbm, phi_hbm, bwo_hbm,
               out_hbm,
               wqk, wv, wo, stage, xtail, xpre, pre, xio, xs, xb, xn, mem_scr, p_scr, o_scr,
               mem0_ref, phi_ref, phi_tab, bqkv_in, bwo_in, bw, bwo, phiq, kv_acc, ob,
               stage_sem, misc_sem, out_sem):

        tail_cp = pltpu.make_async_copy(
            x_hbm.at[pl.ds(0, _LIGHT), pl.ds(KEEP, _SUB)], xtail, misc_sem.at[0])
        mem0_cp = pltpu.make_async_copy(mem0_hbm, mem0_ref, misc_sem.at[5])
        phi_cp = pltpu.make_async_copy(phi_hbm, phi_ref, misc_sem.at[6])
        head, rest = pl.ds(0, 2 * SPI), pl.ds(2 * SPI, NSEG - 2 * SPI)
        head_cp = pltpu.make_async_copy(x_hbm.at[head], xio.at[head], misc_sem.at[3])
        rest_cp = pltpu.make_async_copy(x_hbm.at[rest], xio.at[rest], misc_sem.at[4])
        bqkv_cp = pltpu.make_async_copy(bqkv_hbm, bqkv_in, misc_sem.at[1])
        bwo_cp = pltpu.make_async_copy(bwo_hbm, bwo_in, misc_sem.at[2])

        def stage_cp(src, g, slot, i):
            rows = pl.ds(pl.multiple_of(g * PW, PW), PW)
            return pltpu.make_async_copy(src.at[rows], stage.at[slot, i], stage_sem.at[slot, i])

        def qkv_cps(g):
            return [stage_cp(src, g, g % _RING, i)
                    for i, src in enumerate((wq_hbm, wk_hbm, wv_hbm))]

        def wo_cp(g):
            return stage_cp(wo_hbm, g, (g + 1) % _RING, 3)

        phi_cp.start()
        tail_cp.start()
        for cp in qkv_cps(0):
            cp.start()
        phi_cp.wait()
        table = None
        for d in range(FB):
            sel = jnp.where(_iota((HB, D), 1) == _iota((HB, D), 0) * FB + d, 1.0, 0.0)
            table = _add(table, _mm(phi_ref[d].astype(_F32), sel.astype(_BF)))
        dup = jnp.where(_iota((GR, FB), 0) // 2 == _iota((GR, FB), 1), 1.0, 0.0)
        phi_tab[...] = _mm(dup, table.astype(_BF))
        with jax.named_scope("tailwait"):
            tail_cp.wait()
        xpre[...] = _pack(_layernorm(xtail[...].astype(_F32).reshape(_LIGHT * _SUB, D)))
        for g in range(1, _RING - 1):
            for cp in qkv_cps(g) + [wo_cp(g - 1)]:
                cp.start()

        def load_pair(g, carry):
            nxt = g + _RING - 1

            @pl.when(nxt < NP)
            def _():
                for cp in qkv_cps(nxt):
                    cp.start()

            @pl.when(nxt <= NP)
            def _():
                wo_cp(nxt - 1).start()

            @pl.when(nxt == NP)
            def _():
                head_cp.start()
                mem0_cp.start()

            slot = g % _RING
            prev = jnp.maximum(g - 1, 0)
            for cp in qkv_cps(g):
                cp.wait()
            pl.when(g > 0)(wo_cp(prev).wait)
            wo[prev] = _pack(stage[slot, jnp.where(g > 0, 3, 0)])
            lhs = _unpack(xpre[...])
            ws = [stage[slot, i].T for i in range(3)]
            wqk[g, :, :PW] = _pack(ws[0])
            wqk[g, :, PW:] = _pack(ws[1])
            wv[g] = _pack(ws[2])
            pre[g, :, :PW] = _mm(lhs, stage[slot, 0], _NT)
            pre[g, :, PW:2 * PW] = _mm(lhs, stage[slot, 1], _NT)
            w = _unpack(wv[g])
            pre[g, :, 2 * PW:] = _mm(lhs, w)
            return carry

        with jax.named_scope("load"):
            lax.fori_loop(0, NP, load_pair, 0)
        rest_cp.start()
        bqkv_cp.start()
        bwo_cp.start()
        wo_cp(NP - 1).wait()
        wo[NP - 1] = _pack(stage[NP % _RING, 3])
        head_cp.wait()
        mem0_cp.wait()
        xs[0:SPI] = xio[0:SPI].astype(_F32)

        def prep_b_weights():
            bqkv_cp.wait()
            bwo_cp.wait()
            t = phi_tab[...]
            off = _iota((GR, D), 1) - (_iota((GR, D), 0) % 2) * FB
            phi_t = [jnp.where((off >= g * GR) & (off < g * GR + FB), t, 0.0) for g in range(NG)]
            bw[2] = _pack(bqkv_in[:, 2 * D:].T)
            bwo[...] = _pack(bwo_in[...])
            for part in range(2):
                acc = [None] * NG
                for j in range(D // _LANES):
                    lo, hi = j * _LANES, (j + 1) * _LANES
                    gs = range(lo // GR, (hi - 1) // GR + 1)
                    lhs = jnp.concatenate([phi_t[g][:, lo:hi] for g in gs], axis=0)
                    r = _mm(lhs, bqkv_in[:, part * D + lo:part * D + hi], _NT)
                    for i, g in enumerate(gs):
                        piece = r[i * GR:(i + 1) * GR]
                        acc[g] = piece if acc[g] is None else acc[g] + piece
                bw[part] = _pack(jnp.concatenate(acc, axis=0) * _LOG2E)

        def xb_rows(s, n):
            return pl.ds(pl.multiple_of(s * (SEG // 2), SEG // 2), n * (SEG // 2))

        def tile(i):
            return slice(i * _LANES, (i + 1) * _LANES)

        def packed_tile(i):
            return slice(i * _LANES // 2, (i + 1) * _LANES // 2)

        def a_step(s, mem, light):
            h = jnp.concatenate([mem, xn[s % 2, :KEEP if light else SEG]], axis=0)
            if light:
                h = h.astype(_BF)
            xn[(s + 1) % 2] = _layernorm(xs[jnp.minimum(s + 1, NSEG - 1)])
            prev = jnp.maximum(s - 1, 0)
            xb[xb_rows(prev, 1), :] = _pack(_layernorm(xs[prev]))
            qk = None
            for k in range(D // _LANES):
                qk = _add(qk, _mm(h[:, tile(k)], _unpack(wqk[0, packed_tile(k), :])))
            out = a_light(s, h, qk) if light else a_full(h, qk)
            xs[s] = xs[s] + out[M:]
            return out[:M]

        def scores(g, qk):
            p_scr[g] = pair_softmax(_mm(qk[:, :PW], expand(qk[:, PW:]), _NT))

        def a_full(h, cur):
            for g in range(NP):
                nxt = _mm(h, _unpack(wqk[g + 1] if g + 1 < NP else wv[0]))
                scores(g, cur)
                cur = nxt
            out = None
            for g in range(NP + _LAG):
                if g + 1 < NP:
                    nxt = _mm(h, _unpack(wv[g + 1]))
                if g < NP:
                    o_scr[g] = _mm(p_scr[g], expand(cur))
                    cur = nxt
                if g >= _LAG:
                    out = _add(out, _mm(o_scr[g - _LAG], _unpack(wo[g - _LAG])))
            return out

        def a_light(s, h, qk):
            tail = pl.ds(pl.multiple_of(s * _SUB, _SUB), _SUB)
            out = v = None
            for t in range(1, NP + _LAG + 2):
                qk_new, v_new, n_out = [], [], 0
                g = t - 2 - _LAG
                for op in _LIGHT_ORDER:
                    if op == "q" and t < NP:
                        qk_new.append(_mm(h, _unpack(wqk[t, :, tile(len(qk_new))])))
                    elif op == "v" and t - 1 < NP:
                        v_new.append(_mm(h, _unpack(wv[t - 1, :, tile(len(v_new))])))
                    elif op == "s" and t - 1 < NP:
                        scores(t - 1, jnp.concatenate([qk, pre[t - 1, tail, :2 * PW]], axis=0))
                    elif op == "p" and 0 <= t - 2 < NP:
                        full = jnp.concatenate([v, pre[t - 2, tail, 2 * PW:]], axis=0)
                        o_scr[t - 2] = _mm(p_scr[t - 2], expand(full))
                    elif op == "o":
                        if 0 <= g < NP - 1:
                            w = _unpack(wo[g, packed_tile(n_out), :])
                            out = _add(out, _mm(o_scr[g, :, tile(n_out)], w))
                        elif g == NP - 1 and n_out == 0:
                            out = out + _mm(o_scr[g], _unpack(wo[g]))
                        n_out += 1
                if qk_new:
                    qk = jnp.concatenate(qk_new, axis=1)
                if v_new:
                    v = jnp.concatenate(v_new, axis=1)
            return out

        def a_steps(lo, hi, light, unroll):
            def body(i, carry):
                if light:
                    pl.when(i == 1)(rest_cp.wait)
                mem = mem_scr[...]
                for u in range(unroll):
                    mem = a_step(i * unroll + u, mem, light)
                    if light and u == 0:
                        segs = pl.ds(jnp.minimum((i + 1) * SPI, NSEG - SPI), SPI)
                        xs[segs] = xio[segs].astype(_F32)
                mem_scr[...] = mem
                return carry

            lax.fori_loop(lo // unroll, hi // unroll, body, 0)

        def layer_a(n_light):
            xn[0] = _layernorm(xs[0])
            mem_scr[...] = mem0_ref[...].astype(_F32)
            with jax.named_scope("alight"):
                a_steps(0, n_light, True, _UNROLL_LIGHT)
            with jax.named_scope("aloop"):
                a_steps(n_light, NSEG, False, _UNROLL)
            xb[(S - SEG) // 2:, :] = _pack(_layernorm(xs[NSEG - 1]))

        def b_pass1(c, carry):
            xc = _unpack(xb[xb_rows(c * SPC, SPC), :])
            ones = jnp.ones((_SUB, _CHUNK), _F32)

            def project(part, b):
                return _mm(_unpack(bw[part, b * BLK // 2:(b + 1) * BLK // 2, :]), xc, _NT)

            def groups(t):
                return [t[i * GR:(i + 1) * GR] for i in range(BLK // GR)]

            phik, vs = [], []
            for b in range(D // BLK):
                phik += [feature_map(p).astype(_BF) for p in groups(project(1, b))]
            for b in range(D // BLK):
                vs += groups(project(2, b))
            for b in range(D // BLK):
                for i, p in enumerate(groups(project(0, b))):
                    phiq[c, b * (BLK // GR) + i] = _pack(feature_map(p))
            for g in range(NG):
                kv_acc[g] = kv_acc[g] + _mm(jnp.concatenate([vs[g], ones], axis=0), phik[g], _NT)
            return carry

        def out_cp(c):
            segs = pl.ds(c * SPC, SPC)
            return pltpu.make_async_copy(xio.at[segs], out_hbm.at[segs], out_sem.at[c])

        def b_attend(c):
            first = _iota((_SUB, _CHUNK), 0) < _SUB // 2
            outs = []
            for g in range(NG):
                nd = _mm(kv_acc[g], _unpack(phiq[c, g]))
                mixed = 1.0 / (nd[GR:] + 1e-06)
                swapped = pltpu.roll(mixed, _SUB // 2, 0)
                for i in range(GR // _SUB):
                    if (i + 1) * _SUB <= FB:
                        inv = jnp.where(first, mixed, swapped)
                    elif i * _SUB >= FB:
                        inv = jnp.where(first, swapped, mixed)
                    else:
                        inv = mixed
                    outs.append(nd[i * _SUB:(i + 1) * _SUB] * inv)
            return _pack(jnp.concatenate(outs, axis=0).T)

        def layer_b(last):
            kv_acc[...] = jnp.zeros(kv_acc.shape, _F32)
            with jax.named_scope("b1"):
                lax.fori_loop(0, NCH, b_pass1, 0, unroll=_UNROLL_B)
            shape = (GR + _SUB, 2 * GR)
            row = _iota(shape, 0)
            second = ((row >= FB) & (row < GR)) | (row >= GR + _SUB // 2)
            same_head = jnp.where(second, 1, 0) == _iota(shape, 1) % 2
            for g in range(NG):
                kv_acc[g] = jnp.where(same_head, kv_acc[g], 0.0)
            with jax.named_scope("b2"):
                ob[...] = b_attend(0)

                def b_pass2(c, carry):
                    o = _unpack(ob[...])
                    ob[...] = b_attend(jnp.minimum(c + 1, NCH - 1))
                    segs = pl.ds(c * SPC, SPC)
                    y = xs[segs] + _mm(o, _unpack(bwo[...])).reshape(SPC, SEG, D)
                    xs[segs] = y
                    xio[segs] = y.astype(_BF)
                    pl.when(last)(out_cp(c).start)
                    return carry

                lax.fori_loop(0, NCH, b_pass2, 0, unroll=_UNROLL_B)

        def layer_pair(i, carry):
            layer_a(jnp.where(i == 0, _LIGHT, 0))
            with jax.named_scope("prep"):
                pl.when(i == 0)(prep_b_weights)
            layer_b(i == 1)
            return carry

        lax.fori_loop(0, 2, layer_pair, 0)
        for c in range(NCH):
            out_cp(c).wait()

    scratch = [
        pltpu.VMEM((NP, D // 2, 2 * PW), _U32),
        pltpu.VMEM((NP, D // 2, PW), _U32),
        pltpu.VMEM((NP, PW // 2, D), _U32),
        pltpu.VMEM((_RING, 4, PW, D), _BF),
        pltpu.VMEM((_LIGHT, _SUB, D), _BF),
        pltpu.VMEM((_LIGHT * _SUB // 2, D), _U32),
        pltpu.VMEM((NP, _LIGHT * _SUB, 3 * PW), _F32),
        pltpu.VMEM((NSEG, SEG, D), _BF),
        pltpu.VMEM((NSEG, SEG, D), _F32),
        pltpu.VMEM((S // 2, D), _U32),
        pltpu.VMEM((2, SEG, D), _F32),
        pltpu.VMEM((M, D), _F32),
        pltpu.VMEM((NP, L, 2 * L), _F32),
        pltpu.VMEM((NP, L, PW), _F32),
        pltpu.VMEM((M, D), _BF),
        pltpu.VMEM((FB, FB, HB), _BF),
        pltpu.VMEM((GR, D), _F32),
        pltpu.VMEM((D, 3 * D), _BF),
        pltpu.VMEM((D, D), _BF),
        pltpu.VMEM((3, D // 2, D), _U32),
        pltpu.VMEM((D // 2, D), _U32),
        pltpu.VMEM((NCH, NG, GR, _CHUNK), _U32),
        pltpu.VMEM((NG, GR + _SUB, 2 * GR), _F32),
        pltpu.VMEM((_CHUNK // 2, D), _U32),
        pltpu.SemaphoreType.DMA((_RING, 4)),
        pltpu.SemaphoreType.DMA((7,)),
        pltpu.SemaphoreType.DMA((NCH,)),
    ]
    return kernel, scratch


def pallas_interleave_layers__memory_aug_recurrent_mem_tr__linear_kernel_hedgehog__prompt_kernel(
    A_x, A_mem0, A_Wq, A_Wk, A_Wv, A_Wo, A_seg_len, B_x, B_wqkv, B_w_phi, B_wo,
):
    del B_x
    _, S, D = A_x.shape
    M = A_mem0.shape[1]
    _, H, DH = A_Wq.shape
    HB = B_w_phi.shape[0]
    SEG = int(A_seg_len)
    kernel, scratch = _make_kernel(S, D, M, SEG, H, DH, HB)

    def head_major(w):
        return jnp.transpose(w, (1, 2, 0)).reshape(H * DH, D)

    hbm = pl.BlockSpec(memory_space=pl.ANY)
    out = pl.pallas_call(
        kernel,
        out_shape=jax.ShapeDtypeStruct((S // SEG, SEG, D), A_x.dtype),
        in_specs=[hbm] * 9,
        out_specs=hbm,
        scratch_shapes=scratch,
        compiler_params=pltpu.CompilerParams(vmem_limit_bytes=120 * 1024 * 1024, disable_bounds_checks=True),
    )(
        A_x.reshape(S // SEG, SEG, D),
        A_mem0.reshape(M, D),
        head_major(A_Wq),
        head_major(A_Wk),
        head_major(A_Wv),
        A_Wo.reshape(H * DH, D),
        B_wqkv,
        jnp.transpose(B_w_phi, (1, 2, 0)),
        B_wo,
    )
    return out.reshape(A_x.shape)
```

```python
import jax
import jax.numpy as jnp
from jax import lax
import jax.experimental.pallas as pl
import jax.experimental.pallas.tpu as pltpu

_BF = jnp.bfloat16
_F32 = jnp.float32
_U32 = jnp.uint32
_NN = (((1,), (0,)), ((), ()))
_NT = (((1,), (1,)), ((), ()))
_LANES = 128
_SUB = 8
_EPS = 1e-05
_LOG2E = 1.4426950408889634

_RING = 4
_CHUNK = 256
_LIGHT = 40
_UNROLL = 2
_UNROLL_LIGHT = 2
_LAG = 2
_UNROLL_B = 2
_LIGHT_ORDER = "qqqoqsqoqvvovp"


def _mm(a, b, dims=_NN):
    return lax.dot_general(a, b, dims, preferred_element_type=_F32)


def _add(acc, x):
    return x if acc is None else acc + x


def _iota(shape, dim):
    return lax.broadcasted_iota(jnp.int32, shape, dim)


def _pack(x):
    return pltpu.bitcast(x.astype(_BF), _U32)


def _unpack(x):
    return pltpu.bitcast(x, _BF)


def _layernorm(x):
    m = jnp.mean(x, axis=-1, keepdims=True)
    c = x - m
    v = jnp.mean(c * c, axis=-1, keepdims=True)
    return c * lax.rsqrt(v + _EPS)


def _make_kernel(S, D, M, SEG, H, DH, HB):
    L = M + SEG
    NSEG = S // SEG
    NP = H // 2
    PW = 2 * DH
    FB = D // HB
    NG = HB // 2
    GR = 2 * FB
    BLK = 4 * GR
    NCH = S // _CHUNK
    SPC = _CHUNK // SEG
    SPI = 2 * _UNROLL_LIGHT
    KEEP = SEG - _SUB
    scale = DH ** (-0.5)
    split_tile = DH // _LANES
    split_lane = DH % _LANES

    def expand(t):
        zero = jnp.zeros((L, _LANES), _F32)
        in_a = _iota((L, _LANES), 1) < split_lane
        top, bot = [], []
        for j in range(PW // _LANES):
            blk = t[:, j * _LANES:(j + 1) * _LANES]
            if j < split_tile:
                top.append(blk)
                bot.append(zero)
            elif j == split_tile:
                top.append(jnp.where(in_a, blk, 0.0))
                bot.append(jnp.where(in_a, 0.0, blk))
            else:
                top.append(zero)
                bot.append(blk)
        both = [jnp.concatenate(top, axis=1), jnp.concatenate(bot, axis=1)]
        return jnp.concatenate(both, axis=0).astype(_BF)

    def pair_softmax(s):
        row = _iota((L, 2 * L), 0)
        col = _iota((L, 2 * L), 1)
        is_a = col < L
        key = jnp.where(is_a, col, col - L)
        s = jnp.where((row < M) | (row >= key), s * scale, -1000000000.0)
        max_a = jnp.max(jnp.where(is_a, s, -jnp.inf), axis=1, keepdims=True)
        max_b = jnp.max(jnp.where(is_a, -jnp.inf, s), axis=1, keepdims=True)
        e = jnp.exp(s - jnp.where(is_a, max_a, max_b))
        sum_a = jnp.sum(jnp.where(is_a, e, 0.0), axis=1, keepdims=True)
        sum_b = jnp.sum(jnp.where(is_a, 0.0, e), axis=1, keepdims=True)
        return e / jnp.where(is_a, sum_a, sum_b)

    def over_features(op, rows):
        r = rows[0]
        for t in rows[1:]:
            r = op(r, t)
        r = op(r, pltpu.roll(r, 4, 0))
        return op(r, pltpu.roll(r, 2, 0))

    def feature_map(p):
        rows = [p[i * _SUB:(i + 1) * _SUB] for i in range(GR // _SUB)]
        hi = over_features(jnp.maximum, rows)
        lo = over_features(jnp.minimum, rows)
        out = []
        for es in ([jnp.exp2(r - hi) for r in rows], [jnp.exp2(lo - r) for r in rows]):
            inv = 1.0 / over_features(jnp.add, es)
            out += [e * inv for e in es]
        return jnp.concatenate(out, axis=0)

    def kernel(x_hbm, mem0_hbm, wq_hbm, wk_hbm, wv_hbm, wo_hbm, bqkv_hbm, phi_hbm, bwo_hbm,
               out_hbm,
               wqk, wv, wo, stage, xtail, xpre, pre, xio, xs, xb, xn, mem_scr, p_scr, o_scr,
               mem0_ref, phi_ref, phi_tab, bqkv_in, bwo_in, bw, bwo, phiq, kv_acc, ob,
               stage_sem, misc_sem, out_sem):

        tail_cp = pltpu.make_async_copy(
            x_hbm.at[pl.ds(0, _LIGHT), pl.ds(KEEP, _SUB)], xtail, misc_sem.at[0])
        mem0_cp = pltpu.make_async_copy(mem0_hbm, mem0_ref, misc_sem.at[5])
        phi_cp = pltpu.make_async_copy(phi_hbm, phi_ref, misc_sem.at[6])
        head, rest = pl.ds(0, 2 * SPI), pl.ds(2 * SPI, NSEG - 2 * SPI)
        head_cp = pltpu.make_async_copy(x_hbm.at[head], xio.at[head], misc_sem.at[3])
        rest_cp = pltpu.make_async_copy(x_hbm.at[rest], xio.at[rest], misc_sem.at[4])
        bqkv_cp = pltpu.make_async_copy(bqkv_hbm, bqkv_in, misc_sem.at[1])
        bwo_cp = pltpu.make_async_copy(bwo_hbm, bwo_in, misc_sem.at[2])

        def stage_cp(src, g, slot, i):
            rows = pl.ds(pl.multiple_of(g * PW, PW), PW)
            return pltpu.make_async_copy(src.at[rows], stage.at[slot, i], stage_sem.at[slot, i])

        def qkv_cps(g):
            return [stage_cp(src, g, g % _RING, i)
                    for i, src in enumerate((wq_hbm, wk_hbm, wv_hbm))]

        def wo_cp(g):
            return stage_cp(wo_hbm, g, (g + 1) % _RING, 3)

        phi_cp.start()
        tail_cp.start()
        for cp in qkv_cps(0):
            cp.start()
        phi_cp.wait()
        table = None
        for d in range(FB):
            sel = jnp.where(_iota((HB, D), 1) == _iota((HB, D), 0) * FB + d, 1.0, 0.0)
            table = _add(table, _mm(phi_ref[d].astype(_F32), sel.astype(_BF)))
        dup = jnp.where(_iota((GR, FB), 0) // 2 == _iota((GR, FB), 1), 1.0, 0.0)
        phi_tab[...] = _mm(dup, table.astype(_BF))
        with jax.named_scope("tailwait"):
            tail_cp.wait()
        xpre[...] = _pack(_layernorm(xtail[...].astype(_F32).reshape(_LIGHT * _SUB, D)))
        for g in range(1, _RING - 1):
            for cp in qkv_cps(g) + [wo_cp(g - 1)]:
                cp.start()

        def load_pair(g, carry):
            nxt = g + _RING - 1

            @pl.when(nxt < NP)
            def _():
                for cp in qkv_cps(nxt):
                    cp.start()

            @pl.when(nxt <= NP)
            def _():
                wo_cp(nxt - 1).start()

            @pl.when(nxt == NP)
            def _():
                head_cp.start()
                mem0_cp.start()

            slot = g % _RING
            prev = jnp.maximum(g - 1, 0)
            for cp in qkv_cps(g):
                cp.wait()
            pl.when(g > 0)(wo_cp(prev).wait)
            wo[prev] = _pack(stage[slot, jnp.where(g > 0, 3, 0)])
            lhs = _unpack(xpre[...])
            ws = [stage[slot, i].T for i in range(3)]
            wqk[g, :, :PW] = _pack(ws[0])
            wqk[g, :, PW:] = _pack(ws[1])
            wv[g] = _pack(ws[2])
            pre[g, :, :PW] = _mm(lhs, stage[slot, 0], _NT)
            pre[g, :, PW:2 * PW] = _mm(lhs, stage[slot, 1], _NT)
            w = _unpack(wv[g])
            pre[g, :, 2 * PW:] = _mm(lhs, w)
            return carry

        with jax.named_scope("load"):
            lax.fori_loop(0, NP, load_pair, 0)
        rest_cp.start()
        bqkv_cp.start()
        bwo_cp.start()
        wo_cp(NP - 1).wait()
        wo[NP - 1] = _pack(stage[NP % _RING, 3])
        head_cp.wait()
        mem0_cp.wait()
        xs[0:SPI] = xio[0:SPI].astype(_F32)

        def prep_b_weights():
            bqkv_cp.wait()
            bwo_cp.wait()
            t = phi_tab[...]
            off = _iota((GR, D), 1) - (_iota((GR, D), 0) % 2) * FB
            phi_t = [jnp.where((off >= g * GR) & (off < g * GR + FB), t, 0.0) for g in range(NG)]
            bw[2] = _pack(bqkv_in[:, 2 * D:].T)
            bwo[...] = _pack(bwo_in[...])
            for part in range(2):
                acc = [None] * NG
                for j in range(D // _LANES):
                    lo, hi = j * _LANES, (j + 1) * _LANES
                    gs = range(lo // GR, (hi - 1) // GR + 1)
                    lhs = jnp.concatenate([phi_t[g][:, lo:hi] for g in gs], axis=0)
                    r = _mm(lhs, bqkv_in[:, part * D + lo:part * D + hi], _NT)
                    for i, g in enumerate(gs):
                        piece = r[i * GR:(i + 1) * GR]
                        acc[g] = piece if acc[g] is None else acc[g] + piece
                bw[part] = _pack(jnp.concatenate(acc, axis=0) * _LOG2E)

        def xb_rows(s, n):
            return pl.ds(pl.multiple_of(s * (SEG // 2), SEG // 2), n * (SEG // 2))

        def tile(i):
            return slice(i * _LANES, (i + 1) * _LANES)

        def packed_tile(i):
            return slice(i * _LANES // 2, (i + 1) * _LANES // 2)

        def a_step(s, slot, mem, light):
            h = jnp.concatenate([mem, xn[slot, :KEEP if light else SEG]], axis=0)
            if light:
                h = h.astype(_BF)
            xn[1 - slot] = _layernorm(xs[jnp.minimum(s + 1, NSEG - 1)])
            prev = jnp.maximum(s - 1, 0)
            xb[xb_rows(prev, 1), :] = _pack(_layernorm(xs[prev]))
            qk = None
            for k in range(D // _LANES):
                qk = _add(qk, _mm(h[:, tile(k)], _unpack(wqk[0, packed_tile(k), :])))
            out = a_light(s, h, qk) if light else a_full(h, qk)
            xs[s] = xs[s] + out[M:]
            return out[:M]

        def scores(g, qk):
            p_scr[g] = pair_softmax(_mm(qk[:, :PW], expand(qk[:, PW:]), _NT))

        def finish(out, last):
            cols = []
            for j in range(D // _LANES):
                col = out[:, tile(j)]
                for g in range(NP - last, NP):
                    col = col + _mm(o_scr[g], _unpack(wo[g, :, tile(j)]))
                cols.append(col)
            return jnp.concatenate(cols, axis=1)

        def a_full(h, cur):
            for g in range(NP):
                nxt = _mm(h, _unpack(wqk[g + 1] if g + 1 < NP else wv[0]))
                scores(g, cur)
                cur = nxt
            out = None
            for g in range(NP + _LAG):
                if g + 1 < NP:
                    nxt = _mm(h, _unpack(wv[g + 1]))
                if g < NP:
                    o_scr[g] = _mm(p_scr[g], expand(cur))
                    cur = nxt
                if _LAG <= g < NP + _LAG - 2:
                    out = _add(out, _mm(o_scr[g - _LAG], _unpack(wo[g - _LAG])))
            return finish(out, 2)

        def a_light(s, h, qk):
            tail = pl.ds(pl.multiple_of(s * _SUB, _SUB), _SUB)
            out = v = None
            for t in range(1, NP + _LAG + 2):
                qk_new, v_new, n_out = [], [], 0
                g = t - 2 - _LAG
                for op in _LIGHT_ORDER:
                    if op == "q" and t < NP:
                        qk_new.append(_mm(h, _unpack(wqk[t, :, tile(len(qk_new))])))
                    elif op == "v" and t - 1 < NP:
                        v_new.append(_mm(h, _unpack(wv[t - 1, :, tile(len(v_new))])))
                    elif op == "s" and t - 1 < NP:
                        scores(t - 1, jnp.concatenate([qk, pre[t - 1, tail, :2 * PW]], axis=0))
                    elif op == "p" and 0 <= t - 2 < NP:
                        full = jnp.concatenate([v, pre[t - 2, tail, 2 * PW:]], axis=0)
                        o_scr[t - 2] = _mm(p_scr[t - 2], expand(full))
                    elif op == "o":
                        if 0 <= g < NP - 1:
                            w = _unpack(wo[g, packed_tile(n_out), :])
                            out = _add(out, _mm(o_scr[g, :, tile(n_out)], w))
                        n_out += 1
                if qk_new:
                    qk = jnp.concatenate(qk_new, axis=1)
                if v_new:
                    v = jnp.concatenate(v_new, axis=1)
            return finish(out, 1)

        def a_steps(lo, hi, light, unroll):
            def body(i, carry):
                if light:
                    pl.when(i == 1)(rest_cp.wait)
                mem = mem_scr[...]
                for u in range(unroll):
                    mem = a_step(i * unroll + u, u % 2, mem, light)
                    if light and u == 0:
                        segs = pl.ds(jnp.minimum((i + 1) * SPI, NSEG - SPI), SPI)
                        xs[segs] = xio[segs].astype(_F32)
                mem_scr[...] = mem
                return carry

            lax.fori_loop(lo // unroll, hi // unroll, body, 0)

        def layer_a(n_light):
            xn[0] = _layernorm(xs[0])
            mem_scr[...] = mem0_ref[...].astype(_F32)
            with jax.named_scope("alight"):
                a_steps(0, n_light, True, _UNROLL_LIGHT)
            with jax.named_scope("aloop"):
                a_steps(n_light, NSEG, False, _UNROLL)
            xb[(S - SEG) // 2:, :] = _pack(_layernorm(xs[NSEG - 1]))

        def b_pass1(c, carry):
            xc = _unpack(xb[xb_rows(c * SPC, SPC), :])
            ones = jnp.ones((_SUB, _CHUNK), _F32)

            def project(part, b):
                return _mm(_unpack(bw[part, b * BLK // 2:(b + 1) * BLK // 2, :]), xc, _NT)

            def groups(t):
                return [t[i * GR:(i + 1) * GR] for i in range(BLK // GR)]

            phik, vs = [], []
            for b in range(D // BLK):
                phik += [feature_map(p).astype(_BF) for p in groups(project(1, b))]
            for b in range(D // BLK):
                vs += groups(project(2, b))
            for b in range(D // BLK):
                for i, p in enumerate(groups(project(0, b))):
                    phiq[c, b * (BLK // GR) + i] = _pack(feature_map(p))
            for g in range(NG):
                kv_acc[g] = kv_acc[g] + _mm(jnp.concatenate([vs[g], ones], axis=0), phik[g], _NT)
            return carry

        def out_cp(c):
            segs = pl.ds(c * SPC, SPC)
            return pltpu.make_async_copy(xio.at[segs], out_hbm.at[segs], out_sem.at[c])

        def b_attend(c):
            first = _iota((_SUB, _CHUNK), 0) < _SUB // 2
            outs = []
            for g in range(NG):
                nd = _mm(kv_acc[g], _unpack(phiq[c, g]))
                mixed = 1.0 / (nd[GR:] + 1e-06)
                swapped = pltpu.roll(mixed, _SUB // 2, 0)
                for i in range(GR // _SUB):
                    if (i + 1) * _SUB <= FB:
                        inv = jnp.where(first, mixed, swapped)
                    elif i * _SUB >= FB:
                        inv = jnp.where(first, swapped, mixed)
                    else:
                        inv = mixed
                    outs.append(nd[i * _SUB:(i + 1) * _SUB] * inv)
            return _pack(jnp.concatenate(outs, axis=0).T)

        def layer_b(last):
            kv_acc[...] = jnp.zeros(kv_acc.shape, _F32)
            with jax.named_scope("b1"):
                lax.fori_loop(0, NCH, b_pass1, 0, unroll=_UNROLL_B)
            shape = (GR + _SUB, 2 * GR)
            row = _iota(shape, 0)
            second = ((row >= FB) & (row < GR)) | (row >= GR + _SUB // 2)
            same_head = jnp.where(second, 1, 0) == _iota(shape, 1) % 2
            for g in range(NG):
                kv_acc[g] = jnp.where(same_head, kv_acc[g], 0.0)
            with jax.named_scope("b2"):
                ob[...] = b_attend(0)

                def b_pass2(c, carry):
                    o = _unpack(ob[...])
                    ob[...] = b_attend(jnp.minimum(c + 1, NCH - 1))
                    segs = pl.ds(c * SPC, SPC)
                    y = xs[segs] + _mm(o, _unpack(bwo[...])).reshape(SPC, SEG, D)
                    xs[segs] = y
                    xio[segs] = y.astype(_BF)
                    pl.when(last)(out_cp(c).start)
                    return carry

                lax.fori_loop(0, NCH, b_pass2, 0, unroll=4)

        def layer_pair(i, carry):
            layer_a(jnp.where(i == 0, _LIGHT, 0))
            with jax.named_scope("prep"):
                pl.when(i == 0)(prep_b_weights)
            layer_b(i == 1)
            return carry

        lax.fori_loop(0, 2, layer_pair, 0)
        for c in range(NCH):
            out_cp(c).wait()

    scratch = [
        pltpu.VMEM((NP, D // 2, 2 * PW), _U32),
        pltpu.VMEM((NP, D // 2, PW), _U32),
        pltpu.VMEM((NP, PW // 2, D), _U32),
        pltpu.VMEM((_RING, 4, PW, D), _BF),
        pltpu.VMEM((_LIGHT, _SUB, D), _BF),
        pltpu.VMEM((_LIGHT * _SUB // 2, D), _U32),
        pltpu.VMEM((NP, _LIGHT * _SUB, 3 * PW), _F32),
        pltpu.VMEM((NSEG, SEG, D), _BF),
        pltpu.VMEM((NSEG, SEG, D), _F32),
        pltpu.VMEM((S // 2, D), _U32),
        pltpu.VMEM((2, SEG, D), _F32),
        pltpu.VMEM((M, D), _F32),
        pltpu.VMEM((NP, L, 2 * L), _F32),
        pltpu.VMEM((NP, L, PW), _F32),
        pltpu.VMEM((M, D), _BF),
        pltpu.VMEM((FB, FB, HB), _BF),
        pltpu.VMEM((GR, D), _F32),
        pltpu.VMEM((D, 3 * D), _BF),
        pltpu.VMEM((D, D), _BF),
        pltpu.VMEM((3, D // 2, D), _U32),
        pltpu.VMEM((D // 2, D), _U32),
        pltpu.VMEM((NCH, NG, GR, _CHUNK), _U32),
        pltpu.VMEM((NG, GR + _SUB, 2 * GR), _F32),
        pltpu.VMEM((_CHUNK // 2, D), _U32),
        pltpu.SemaphoreType.DMA((_RING, 4)),
        pltpu.SemaphoreType.DMA((7,)),
        pltpu.SemaphoreType.DMA((NCH,)),
    ]
    return kernel, scratch


def pallas_interleave_layers__memory_aug_recurrent_mem_tr__linear_kernel_hedgehog__prompt_kernel(
    A_x, A_mem0, A_Wq, A_Wk, A_Wv, A_Wo, A_seg_len, B_x, B_wqkv, B_w_phi, B_wo,
):
    del B_x
    _, S, D = A_x.shape
    M = A_mem0.shape[1]
    _, H, DH = A_Wq.shape
    HB = B_w_phi.shape[0]
    SEG = int(A_seg_len)
    kernel, scratch = _make_kernel(S, D, M, SEG, H, DH, HB)

    def head_major(w):
        return jnp.transpose(w, (1, 2, 0)).reshape(H * DH, D)

    hbm = pl.BlockSpec(memory_space=pl.ANY)
    out = pl.pallas_call(
        kernel,
        out_shape=jax.ShapeDtypeStruct((S // SEG, SEG, D), A_x.dtype),
        in_specs=[hbm] * 9,
        out_specs=hbm,
        scratch_shapes=scratch,
        compiler_params=pltpu.CompilerParams(vmem_limit_bytes=120 * 1024 * 1024, disable_bounds_checks=True),
    )(
        A_x.reshape(S // SEG, SEG, D),
        A_mem0.reshape(M, D),
        head_major(A_Wq),
        head_major(A_Wk),
        head_major(A_Wv),
        A_Wo.reshape(H * DH, D),
        B_wqkv,
        jnp.transpose(B_w_phi, (1, 2, 0)),
        B_wo,
    )
    return out.reshape(A_x.shape)
```

```python
import jax
import jax.numpy as jnp
from jax import lax
import jax.experimental.pallas as pl
import jax.experimental.pallas.tpu as pltpu

_BF = jnp.bfloat16
_F32 = jnp.float32
_U32 = jnp.uint32
_NN = (((1,), (0,)), ((), ()))
_NT = (((1,), (1,)), ((), ()))
_LANES = 128
_SUB = 8
_EPS = 1e-05
_LOG2E = 1.4426950408889634

_RING = 4
_CHUNK = 256
_LIGHT = 40
_LAG = 2
_LIGHT_ORDER = "qqqqqsoqovvovp"
_UNROLL_A = 2
_UNROLL_KV = 2
_UNROLL_OUT = 4


def _mm(a, b, dims=_NN):
    return lax.dot_general(a, b, dims, preferred_element_type=_F32)


def _add(acc, x):
    return x if acc is None else acc + x


def _iota(shape, dim):
    return lax.broadcasted_iota(jnp.int32, shape, dim)


def _pack(x):
    return pltpu.bitcast(x.astype(_BF), _U32)


def _unpack(x):
    return pltpu.bitcast(x, _BF)


def _layernorm(x):
    m = jnp.mean(x, axis=-1, keepdims=True)
    c = x - m
    v = jnp.mean(c * c, axis=-1, keepdims=True)
    return c * lax.rsqrt(v + _EPS)


def _make_kernel(S, D, M, SEG, H, DH, HB):
    L = M + SEG
    NSEG = S // SEG
    NP = H // 2
    PW = 2 * DH
    FB = D // HB
    NG = HB // 2
    GR = 2 * FB
    BLK = 4 * GR
    NCH = S // _CHUNK
    SPC = _CHUNK // SEG
    SPI = 2 * _UNROLL_A
    KEEP = SEG - _SUB
    scale = DH ** (-0.5)
    split_tile = DH // _LANES
    split_lane = DH % _LANES
    assert M == _SUB and SEG % (2 * _SUB) == 0 and 2 * L <= _LANES and D % _LANES == 0
    assert H % 2 == 0 and PW % _LANES == 0 and NP >= _RING
    assert _LIGHT_ORDER.count("q") * _LANES == 2 * PW and _LIGHT_ORDER.count("v") * _LANES == PW
    assert HB % 2 == 0 and FB % _SUB == _SUB // 2 and D % BLK == 0
    assert S % _CHUNK == 0 and _CHUNK % SEG == 0 and NSEG % SPI == 0
    assert _UNROLL_A % 2 == 0 and _LIGHT % _UNROLL_A == 0 and NSEG // 2 <= _LIGHT < NSEG - SPI

    def expand(t):
        zero = jnp.zeros((L, _LANES), _F32)
        in_a = _iota((L, _LANES), 1) < split_lane
        top, bot = [], []
        for j in range(PW // _LANES):
            blk = t[:, j * _LANES:(j + 1) * _LANES]
            if j < split_tile:
                top.append(blk)
                bot.append(zero)
            elif j == split_tile:
                top.append(jnp.where(in_a, blk, 0.0))
                bot.append(jnp.where(in_a, 0.0, blk))
            else:
                top.append(zero)
                bot.append(blk)
        both = [jnp.concatenate(top, axis=1), jnp.concatenate(bot, axis=1)]
        return jnp.concatenate(both, axis=0).astype(_BF)

    def pair_softmax(s):
        row = _iota((L, 2 * L), 0)
        col = _iota((L, 2 * L), 1)
        is_a = col < L
        key = jnp.where(is_a, col, col - L)
        s = jnp.where((row < M) | (row >= key), s * scale, -1000000000.0)
        max_a = jnp.max(jnp.where(is_a, s, -jnp.inf), axis=1, keepdims=True)
        max_b = jnp.max(jnp.where(is_a, -jnp.inf, s), axis=1, keepdims=True)
        e = jnp.exp(s - jnp.where(is_a, max_a, max_b))
        sum_a = jnp.sum(jnp.where(is_a, e, 0.0), axis=1, keepdims=True)
        sum_b = jnp.sum(jnp.where(is_a, 0.0, e), axis=1, keepdims=True)
        return e / jnp.where(is_a, sum_a, sum_b)

    def over_features(op, rows):
        r = rows[0]
        for t in rows[1:]:
            r = op(r, t)
        r = op(r, pltpu.roll(r, 4, 0))
        return op(r, pltpu.roll(r, 2, 0))

    def feature_map(p):
        rows = [p[i * _SUB:(i + 1) * _SUB] for i in range(GR // _SUB)]
        hi = over_features(jnp.maximum, rows)
        lo = over_features(jnp.minimum, rows)
        out = []
        for es in ([jnp.exp2(r - hi) for r in rows], [jnp.exp2(lo - r) for r in rows]):
            inv = 1.0 / over_features(jnp.add, es)
            out += [e * inv for e in es]
        return jnp.concatenate(out, axis=0)

    def kernel(x_hbm, mem0_hbm, wq_hbm, wk_hbm, wv_hbm, wo_hbm, bqkv_hbm, phi_hbm, bwo_hbm,
               out_hbm,
               wqk, wv, wo, stage, xtail, xpre, pre, xio, xs, xb, xn, mem_scr, p_scr, o_scr,
               mem0_ref, phi_ref, phi_tab, bqkv_in, bwo_in, bw, bwo, phiq, kv_acc, ob,
               stage_sem, misc_sem, out_sem):

        tail_cp = pltpu.make_async_copy(
            x_hbm.at[pl.ds(0, _LIGHT), pl.ds(KEEP, _SUB)], xtail, misc_sem.at[0])
        mem0_cp = pltpu.make_async_copy(mem0_hbm, mem0_ref, misc_sem.at[5])
        phi_cp = pltpu.make_async_copy(phi_hbm, phi_ref, misc_sem.at[6])
        head, rest = pl.ds(0, 2 * SPI), pl.ds(2 * SPI, NSEG - 2 * SPI)
        head_cp = pltpu.make_async_copy(x_hbm.at[head], xio.at[head], misc_sem.at[3])
        rest_cp = pltpu.make_async_copy(x_hbm.at[rest], xio.at[rest], misc_sem.at[4])
        bqkv_cp = pltpu.make_async_copy(bqkv_hbm, bqkv_in, misc_sem.at[1])
        bwo_cp = pltpu.make_async_copy(bwo_hbm, bwo_in, misc_sem.at[2])

        def stage_cp(src, g, slot, i):
            rows = pl.ds(pl.multiple_of(g * PW, PW), PW)
            return pltpu.make_async_copy(src.at[rows], stage.at[slot, i], stage_sem.at[slot, i])

        def qkv_cps(g):
            return [stage_cp(src, g, g % _RING, i)
                    for i, src in enumerate((wq_hbm, wk_hbm, wv_hbm))]

        def wo_cp(g):
            return stage_cp(wo_hbm, g, (g + 1) % _RING, 3)

        phi_cp.start()
        tail_cp.start()
        for cp in qkv_cps(0):
            cp.start()
        phi_cp.wait()
        table = None
        for d in range(FB):
            sel = jnp.where(_iota((HB, D), 1) == _iota((HB, D), 0) * FB + d, 1.0, 0.0)
            table = _add(table, _mm(phi_ref[d].astype(_F32), sel.astype(_BF)))
        dup = jnp.where(_iota((GR, FB), 0) // 2 == _iota((GR, FB), 1), 1.0, 0.0)
        phi_tab[...] = _mm(dup, table.astype(_BF))
        tail_cp.wait()
        xpre[...] = _pack(_layernorm(xtail[...].astype(_F32).reshape(_LIGHT * _SUB, D)))
        for g in range(1, _RING - 1):
            for cp in qkv_cps(g) + [wo_cp(g - 1)]:
                cp.start()

        def load_pair(g, carry):
            nxt = g + _RING - 1

            @pl.when(nxt < NP)
            def _():
                for cp in qkv_cps(nxt):
                    cp.start()

            @pl.when(nxt <= NP)
            def _():
                wo_cp(nxt - 1).start()

            @pl.when(nxt == NP)
            def _():
                head_cp.start()
                mem0_cp.start()

            slot = g % _RING
            prev = jnp.maximum(g - 1, 0)
            for cp in qkv_cps(g):
                cp.wait()
            pl.when(g > 0)(wo_cp(prev).wait)
            wo[prev] = _pack(stage[slot, jnp.where(g > 0, 3, 0)])
            lhs = _unpack(xpre[...])
            ws = [stage[slot, i].T for i in range(3)]
            wqk[g, :, :PW] = _pack(ws[0])
            wqk[g, :, PW:] = _pack(ws[1])
            wv[g] = _pack(ws[2])
            pre[g, :, :PW] = _mm(lhs, stage[slot, 0], _NT)
            pre[g, :, PW:2 * PW] = _mm(lhs, stage[slot, 1], _NT)
            w = _unpack(wv[g])
            pre[g, :, 2 * PW:] = _mm(lhs, w)
            return carry

        lax.fori_loop(0, NP, load_pair, 0)
        rest_cp.start()
        bqkv_cp.start()
        bwo_cp.start()
        wo_cp(NP - 1).wait()
        wo[NP - 1] = _pack(stage[NP % _RING, 3])
        head_cp.wait()
        mem0_cp.wait()
        xs[0:SPI] = xio[0:SPI].astype(_F32)

        def prep_b_weights():
            bqkv_cp.wait()
            bwo_cp.wait()
            t = phi_tab[...]
            off = _iota((GR, D), 1) - (_iota((GR, D), 0) % 2) * FB
            phi_t = [jnp.where((off >= g * GR) & (off < g * GR + FB), t, 0.0) for g in range(NG)]
            bw[2] = _pack(bqkv_in[:, 2 * D:].T)
            bwo[...] = _pack(bwo_in[...])
            for part in range(2):
                acc = [None] * NG
                for j in range(D // _LANES):
                    lo, hi = j * _LANES, (j + 1) * _LANES
                    gs = range(lo // GR, (hi - 1) // GR + 1)
                    lhs = jnp.concatenate([phi_t[g][:, lo:hi] for g in gs], axis=0)
                    r = _mm(lhs, bqkv_in[:, part * D + lo:part * D + hi], _NT)
                    for i, g in enumerate(gs):
                        piece = r[i * GR:(i + 1) * GR]
                        acc[g] = piece if acc[g] is None else acc[g] + piece
                bw[part] = _pack(jnp.concatenate(acc, axis=0) * _LOG2E)

        def xb_rows(s, n):
            return pl.ds(pl.multiple_of(s * (SEG // 2), SEG // 2), n * (SEG // 2))

        def tile(i):
            return slice(i * _LANES, (i + 1) * _LANES)

        def packed_tile(i):
            return slice(i * _LANES // 2, (i + 1) * _LANES // 2)

        def a_step(s, slot, mem, light):
            h = jnp.concatenate([mem, xn[slot, :KEEP if light else SEG]], axis=0)
            if light:
                h = h.astype(_BF)
            xn[1 - slot] = _layernorm(xs[jnp.minimum(s + 1, NSEG - 1)])
            prev = jnp.maximum(s - 1, 0)
            xb[xb_rows(prev, 1), :] = _pack(_layernorm(xs[prev]))
            qk = None
            for k in range(D // _LANES):
                qk = _add(qk, _mm(h[:, tile(k)], _unpack(wqk[0, packed_tile(k), :])))
            out = a_light(s, h, qk) if light else a_full(h, qk)
            xs[s] = xs[s] + out[M:]
            return out[:M]

        def scores(g, qk):
            p_scr[g] = pair_softmax(_mm(qk[:, :PW], expand(qk[:, PW:]), _NT))

        def finish(out, last):
            cols = []
            for j in range(D // _LANES):
                col = out[:, tile(j)]
                for g in range(NP - last, NP):
                    col = col + _mm(o_scr[g], _unpack(wo[g, :, tile(j)]))
                cols.append(col)
            return jnp.concatenate(cols, axis=1)

        def a_full(h, cur):
            for g in range(NP):
                nxt = _mm(h, _unpack(wqk[g + 1] if g + 1 < NP else wv[0]))
                scores(g, cur)
                cur = nxt
            out = None
            for g in range(NP + _LAG):
                if g + 1 < NP:
                    nxt = _mm(h, _unpack(wv[g + 1]))
                if g < NP:
                    o_scr[g] = _mm(p_scr[g], expand(cur))
                    cur = nxt
                if _LAG <= g < NP + _LAG - 2:
                    out = _add(out, _mm(o_scr[g - _LAG], _unpack(wo[g - _LAG])))
            return finish(out, 2)

        def a_light(s, h, qk):
            tail = pl.ds(pl.multiple_of(s * _SUB, _SUB), _SUB)
            out = v = None
            for t in range(1, NP + _LAG + 2):
                qk_new, v_new, n_out = [], [], 0
                g = t - 2 - _LAG
                for op in _LIGHT_ORDER:
                    if op == "q" and t < NP:
                        qk_new.append(_mm(h, _unpack(wqk[t, :, tile(len(qk_new))])))
                    elif op == "v" and t - 1 < NP:
                        v_new.append(_mm(h, _unpack(wv[t - 1, :, tile(len(v_new))])))
                    elif op == "s" and t - 1 < NP:
                        scores(t - 1, jnp.concatenate([qk, pre[t - 1, tail, :2 * PW]], axis=0))
                    elif op == "p" and 0 <= t - 2 < NP:
                        full = jnp.concatenate([v, pre[t - 2, tail, 2 * PW:]], axis=0)
                        o_scr[t - 2] = _mm(p_scr[t - 2], expand(full))
                    elif op == "o":
                        if 0 <= g < NP - 1:
                            w = _unpack(wo[g, packed_tile(n_out), :])
                            out = _add(out, _mm(o_scr[g, :, tile(n_out)], w))
                        n_out += 1
                if qk_new:
                    qk = jnp.concatenate(qk_new, axis=1)
                if v_new:
                    v = jnp.concatenate(v_new, axis=1)
            return finish(out, 1)

        def a_steps(lo, hi, light):
            def body(i, carry):
                if light:
                    pl.when(i == 1)(rest_cp.wait)
                mem = mem_scr[...]
                for u in range(_UNROLL_A):
                    mem = a_step(i * _UNROLL_A + u, u % 2, mem, light)
                    if light and u == 0:
                        segs = pl.ds(jnp.minimum((i + 1) * SPI, NSEG - SPI), SPI)
                        xs[segs] = xio[segs].astype(_F32)
                mem_scr[...] = mem
                return carry

            lax.fori_loop(lo // _UNROLL_A, hi // _UNROLL_A, body, 0)

        def layer_a(n_light):
            xn[0] = _layernorm(xs[0])
            mem_scr[...] = mem0_ref[...].astype(_F32)
            a_steps(0, n_light, True)
            a_steps(n_light, NSEG, False)
            xb[(S - SEG) // 2:, :] = _pack(_layernorm(xs[NSEG - 1]))

        def b_pass1(c, carry):
            xc = _unpack(xb[xb_rows(c * SPC, SPC), :])
            ones = jnp.ones((_SUB, _CHUNK), _F32)

            def project(part, b):
                return _mm(_unpack(bw[part, b * BLK // 2:(b + 1) * BLK // 2, :]), xc, _NT)

            def groups(t):
                return [t[i * GR:(i + 1) * GR] for i in range(BLK // GR)]

            phik, vs = [], []
            for b in range(D // BLK):
                phik += [feature_map(p).astype(_BF) for p in groups(project(1, b))]
            for b in range(D // BLK):
                vs += groups(project(2, b))
            for b in range(D // BLK):
                for i, p in enumerate(groups(project(0, b))):
                    phiq[c, b * (BLK // GR) + i] = _pack(feature_map(p))
            for g in range(NG):
                kv_acc[g] = kv_acc[g] + _mm(jnp.concatenate([vs[g], ones], axis=0), phik[g], _NT)
            return carry

        def out_cp(c):
            segs = pl.ds(c * SPC, SPC)
            return pltpu.make_async_copy(xio.at[segs], out_hbm.at[segs], out_sem.at[c])

        def b_attend(c):
            first = _iota((_SUB, _CHUNK), 0) < _SUB // 2
            outs = []
            for g in range(NG):
                nd = _mm(kv_acc[g], _unpack(phiq[c, g]))
                mixed = 1.0 / (nd[GR:] + 1e-06)
                swapped = pltpu.roll(mixed, _SUB // 2, 0)
                for i in range(GR // _SUB):
                    if (i + 1) * _SUB <= FB:
                        inv = jnp.where(first, mixed, swapped)
                    elif i * _SUB >= FB:
                        inv = jnp.where(first, swapped, mixed)
                    else:
                        inv = mixed
                    outs.append(nd[i * _SUB:(i + 1) * _SUB] * inv)
            return _pack(jnp.concatenate(outs, axis=0).T)

        def layer_b(last):
            kv_acc[...] = jnp.zeros(kv_acc.shape, _F32)
            lax.fori_loop(0, NCH, b_pass1, 0, unroll=_UNROLL_KV)
            shape = (GR + _SUB, 2 * GR)
            row = _iota(shape, 0)
            second = ((row >= FB) & (row < GR)) | (row >= GR + _SUB // 2)
            same_head = jnp.where(second, 1, 0) == _iota(shape, 1) % 2
            for g in range(NG):
                kv_acc[g] = jnp.where(same_head, kv_acc[g], 0.0)
            ob[...] = b_attend(0)

            def b_pass2(c, carry):
                o = _unpack(ob[...])
                ob[...] = b_attend(jnp.minimum(c + 1, NCH - 1))
                segs = pl.ds(c * SPC, SPC)
                y = xs[segs] + _mm(o, _unpack(bwo[...])).reshape(SPC, SEG, D)
                xs[segs] = y
                xio[segs] = y.astype(_BF)
                pl.when(last)(out_cp(c).start)
                return carry

            lax.fori_loop(0, NCH, b_pass2, 0, unroll=_UNROLL_OUT)

        def layer_pair(i, carry):
            layer_a(jnp.where(i == 0, _LIGHT, 0))
            pl.when(i == 0)(prep_b_weights)
            layer_b(i == 1)
            return carry

        lax.fori_loop(0, 2, layer_pair, 0)
        for c in range(NCH):
            out_cp(c).wait()

    scratch = [
        pltpu.VMEM((NP, D // 2, 2 * PW), _U32),
        pltpu.VMEM((NP, D // 2, PW), _U32),
        pltpu.VMEM((NP, PW // 2, D), _U32),
        pltpu.VMEM((_RING, 4, PW, D), _BF),
        pltpu.VMEM((_LIGHT, _SUB, D), _BF),
        pltpu.VMEM((_LIGHT * _SUB // 2, D), _U32),
        pltpu.VMEM((NP, _LIGHT * _SUB, 3 * PW), _F32),
        pltpu.VMEM((NSEG, SEG, D), _BF),
        pltpu.VMEM((NSEG, SEG, D), _F32),
        pltpu.VMEM((S // 2, D), _U32),
        pltpu.VMEM((2, SEG, D), _F32),
        pltpu.VMEM((M, D), _F32),
        pltpu.VMEM((NP, L, 2 * L), _F32),
        pltpu.VMEM((NP, L, PW), _F32),
        pltpu.VMEM((M, D), _BF),
        pltpu.VMEM((FB, FB, HB), _BF),
        pltpu.VMEM((GR, D), _F32),
        pltpu.VMEM((D, 3 * D), _BF),
        pltpu.VMEM((D, D), _BF),
        pltpu.VMEM((3, D // 2, D), _U32),
        pltpu.VMEM((D // 2, D), _U32),
        pltpu.VMEM((NCH, NG, GR, _CHUNK), _U32),
        pltpu.VMEM((NG, GR + _SUB, 2 * GR), _F32),
        pltpu.VMEM((_CHUNK // 2, D), _U32),
        pltpu.SemaphoreType.DMA((_RING, 4)),
        pltpu.SemaphoreType.DMA((7,)),
        pltpu.SemaphoreType.DMA((NCH,)),
    ]
    return kernel, scratch


def pallas_interleave_layers__memory_aug_recurrent_mem_tr__linear_kernel_hedgehog__prompt_kernel(
    A_x, A_mem0, A_Wq, A_Wk, A_Wv, A_Wo, A_seg_len, B_x, B_wqkv, B_w_phi, B_wo,
):
    del B_x
    _, S, D = A_x.shape
    M = A_mem0.shape[1]
    _, H, DH = A_Wq.shape
    HB = B_w_phi.shape[0]
    SEG = int(A_seg_len)
    kernel, scratch = _make_kernel(S, D, M, SEG, H, DH, HB)

    def head_major(w):
        return jnp.transpose(w, (1, 2, 0)).reshape(H * DH, D)

    hbm = pl.BlockSpec(memory_space=pl.ANY)
    out = pl.pallas_call(
        kernel,
        out_shape=jax.ShapeDtypeStruct((S // SEG, SEG, D), A_x.dtype),
        in_specs=[hbm] * 9,
        out_specs=hbm,
        scratch_shapes=scratch,
        compiler_params=pltpu.CompilerParams(vmem_limit_bytes=120 * 1024 * 1024),
    )(
        A_x.reshape(S // SEG, SEG, D),
        A_mem0.reshape(M, D),
        head_major(A_Wq),
        head_major(A_Wk),
        head_major(A_Wv),
        A_Wo.reshape(H * DH, D),
        B_wqkv,
        jnp.transpose(B_w_phi, (1, 2, 0)),
        B_wo,
    )
    return out.reshape(A_x.shape)
```
